```python
import os as _os
_os.environ.setdefault("JAX_PLATFORMS", "cpu")
import jax
import jax.numpy as jnp

def _softmax(x, axis=-1):
    return jax.nn.softmax(x, axis=axis)
def _gelu(x):
    return jax.nn.gelu(x, approximate=True)
def _silu(x):
    return jax.nn.silu(x)
def _sigmoid(x):
    return jax.nn.sigmoid(x)
def _layernorm(x, axis=-1, eps=1e-5):
    m = jnp.mean(x, axis=axis, keepdims=True)
    v = jnp.var(x, axis=axis, keepdims=True)
    return (x - m) / jnp.sqrt(v + eps)
def _scatter_add(tgt, idx, src, axis=0):
    return tgt.at[idx].add(src)
def _segment_sum(src, seg, n):
    return jax.ops.segment_sum(src, seg, n)
class _Rng:
    def __init__(self, key):
        self._k = key
    def _next(self):
        self._k, sub = jax.random.split(self._k)
        return sub
    def normal(self, shape):
        return jax.random.normal(self._next(), shape, dtype=jnp.bfloat16)
    def randint(self, lo, hi, shape):
        return jax.random.randint(self._next(), shape, lo, hi, dtype=jnp.int32)
    def uniform(self, shape, lo=0.0, hi=1.0):
        return jax.random.uniform(self._next(), shape, jnp.bfloat16, lo, hi)
    def permutation(self, n):
        return jax.random.permutation(self._next(), n)


kernel_name = 'gated_mix__grouped_kv_mqa__glu_gated_reglu__prompt'

def setup_inputs():
    _rng = _Rng(jax.random.key(int.from_bytes(__import__("os").urandom(4), "little")))
    _w = (lambda a: (lambda t: t.astype(jnp.bfloat16) if jnp.issubdtype(t.dtype, jnp.floating) else t)(jnp.asarray(a)))
    def _A_setup():
        B, S, D, H = 1, 2048, 1024, 32
        Dh = D // H
        return {
            "x": _w((lambda *s: _rng.normal(s) * 0.05)(B, S, D)),
            "wq": _w((lambda *s: _rng.normal(s) * 0.2)(D, H * Dh)),
            "wk": _w((lambda *s: _rng.normal(s) * 0.2)(D, Dh)),
            "wv": _w((lambda *s: _rng.normal(s) * 0.05)(D, Dh)),
            "wo": _w((lambda *s: _rng.normal(s) * 0.05)(H * Dh, D)),
        }
    _A_in = _A_setup()

    def _B_setup():
        B, S, D, F = 1, 2048, 1024, 3584
        return {
            "x": _w((lambda *s: _rng.normal(s) * 0.05)(B, S, D)),
            "W_gate": _w((lambda *s: _rng.normal(s) * 0.8)(D, F) * (2.0 / D) ** 0.5),
            "W_up": _w((lambda *s: _rng.normal(s) * 0.8)(D, F) * (2.0 / D) ** 0.5),
            "W_down": _w((lambda *s: _rng.normal(s) * 0.8)(F, D) * (1.0 / F) ** 0.5),
        }
    _B_in = _B_setup()

    return {
        "A_x": _A_in["x"],
        "A_wq": _A_in["wq"],
        "A_wk": _A_in["wk"],
        "A_wv": _A_in["wv"],
        "A_wo": _A_in["wo"],
        "B_x": _B_in["x"],
        "B_W_gate": _B_in["W_gate"],
        "B_W_up": _B_in["W_up"],
        "B_W_down": _B_in["W_down"],
        "gate_w": _w((lambda *s: _rng.normal(s) * 0.05)(1024) * 16.0),
    }

def reference(A_x, A_wq, A_wk, A_wv, A_wo, B_x, B_W_gate, B_W_up, B_W_down, gate_w):
    def _A_ref(x, wq, wk, wv, wo):
        B, S, D = x.shape
        H = 32
        Dh = D // H
        q = (lambda x, *d: x.transpose(*d))((x @ wq).reshape(B, S, H, Dh), 0, 2, 1, 3)
        k = x @ wk
        v = x @ wv
        scores = jnp.einsum("bhqd,bkd->bhqk", q, k) * (Dh ** -0.5)
        p = _softmax(scores, axis=-1)
        o = jnp.einsum("bhqk,bkd->bhqd", p, v)
        return (lambda x, *d: x.transpose(*d))(o, 0, 2, 1, 3).reshape(B, S, H * Dh) @ wo

    def _B_ref(x, W_gate, W_up, W_down):
        gate = jnp.einsum("bsd,df->bsf", x, W_gate)
        up = jnp.einsum("bsd,df->bsf", x, W_up)
        gate = gate * (lambda x, dt: x.astype(dt))(gate > 0, gate.dtype)
        h = gate * up
        return jnp.einsum("bsf,fd->bsd", h, W_down)

    x = A_x
    g = _sigmoid((x * gate_w).sum(-1, keepdims=True))
    a = _A_ref(x, A_wq, A_wk, A_wv, A_wo)
    b = _B_ref(x, B_W_gate, B_W_up, B_W_down)
    return g * a + (1 - g) * b
```

```python
import math

import jax
import jax.numpy as jnp
from jax import lax
import jax.experimental.pallas as pl
import jax.experimental.pallas.tpu as pltpu

_F32 = jnp.float32
_BF16 = jnp.bfloat16

_TM = 512
_TP = 512
_W = 512
_KC = 128
_G = 4
_FC = 512
_FS = 256


def _make_kernel(S, D, H, Dh, F):
    NQ = S // _W
    NB = H * NQ
    NC = S // _KC
    NX = S // _TP
    G = _G
    W = _W
    KC = _KC
    q_scale = (Dh ** -0.5) * math.log2(math.e)

    def kernel(x_hbm, wq_hbm, wk_hbm, wv_hbm, wo_hbm, wg_hbm, wu_hbm, wd_hbm, gw_hbm,
               out_ref,
               x_v, wq_v, wk_v, wv_v, wo_v, wg_v, wu_v, wd_v, gw_v,
               qt_v, k_v, vt_v, ot_v, acc_v, sems, *bufs):
        sbufs = bufs[:2 * G]
        mbufs = bufs[2 * G:]
        step_id = pl.program_id(0)

        def x_copy(i):
            return pltpu.make_async_copy(
                x_hbm.at[pl.ds(i * _TP, _TP)], x_v.at[pl.ds(i * _TP, _TP)], sems.at[i])

        w_pairs = [(wk_hbm, wk_v), (wv_hbm, wv_v), (wq_hbm, wq_v), (gw_hbm, gw_v),
                   (wo_hbm, wo_v), (wg_hbm, wg_v), (wu_hbm, wu_v), (wd_hbm, wd_v)]

        def w_copy(j):
            return pltpu.make_async_copy(w_pairs[j][0], w_pairs[j][1], sems.at[NX + j])

        def blk_idx(b):
            h = b // NQ
            qi = b % NQ
            return (pl.ds(pl.multiple_of(h * Dh, Dh), Dh), pl.ds(pl.multiple_of(qi * W, W), W))

        def attn_step(b_next, b_cur, s_next, m_next, s_cur, m_cur):
            do_qk = b_next is not None
            do_pv = b_cur is not None
            if do_qk:
                qt = qt_v[blk_idx(b_next)]
                mx = None
            if do_pv:
                m = jnp.broadcast_to(m_cur[...], (8, W))
                acc = jnp.zeros((Dh, W), _F32)
                l = jnp.zeros((8, W), _F32)
            for c in range(NC):
                rows = slice(c * KC, (c + 1) * KC)
                if do_qk:
                    s = jnp.dot(k_v[rows, :], qt, preferred_element_type=_F32)
                    s_next[rows, :] = s
                    cm = jnp.max(s.reshape(KC // 8, 8, W), axis=0)
                    mx = cm if mx is None else jnp.maximum(mx, cm)
                if do_pv:
                    sc = s_cur[rows, :].reshape(KC // 8, 8, W)
                    p = jnp.exp2(sc - m[None])
                    l = l + jnp.sum(p, axis=0)
                    pb = p.reshape(KC, W).astype(_BF16)
                    acc = acc + jnp.dot(vt_v[:, rows], pb, preferred_element_type=_F32)
            if do_qk:
                m_next[...] = jnp.max(mx, axis=0, keepdims=True)
            if do_pv:
                lt = jnp.sum(l, axis=0, keepdims=True)
                ot_v[blk_idx(b_cur)] = (acc * (1.0 / lt)).astype(_BF16)

        @pl.when(step_id == 0)
        def _prologue_and_attention():
            x_copy(0).start()
            for j in range(3):
                w_copy(j).start()
            for i in range(1, NX):
                x_copy(i).start()
            for j in range(3, len(w_pairs)):
                w_copy(j).start()

            for j in range(3):
                w_copy(j).wait()
            for i in range(NX):
                x_copy(i).wait()
                rows = slice(i * _TP, (i + 1) * _TP)
                xt = x_v[rows, :]
                k_v[rows, :] = jnp.dot(xt, wk_v[...], preferred_element_type=_F32).astype(_BF16)
                v = jnp.dot(xt, wv_v[...], preferred_element_type=_F32)
                vt_v[:, rows] = v.T.astype(_BF16)
                q = jnp.dot(xt, wq_v[...], preferred_element_type=_F32) * q_scale
                qt_v[:, rows] = q.T.astype(_BF16)

            for g in range(G):
                attn_step(g, None, sbufs[g], mbufs[g], None, None)

            def body(i, carry):
                for par in range(2):
                    @pl.when(i % 2 == par)
                    def _():
                        for g in range(G):
                            cur = par * G + g
                            nxt = (1 - par) * G + g
                            b = i * G + g
                            attn_step(b + G, b, sbufs[nxt], mbufs[nxt], sbufs[cur], mbufs[cur])
                return carry

            n_it = NB // G
            lax.fori_loop(0, n_it - 1, body, 0)
            par = (n_it - 1) % 2
            for g in range(G):
                cur = par * G + g
                attn_step(None, (n_it - 1) * G + g, None, None, sbufs[cur], mbufs[cur])

            for j in range(3, len(w_pairs)):
                w_copy(j).wait()

        r0 = pl.multiple_of(step_id * _TM, _TM)
        rows = pl.ds(r0, _TM)

        acc_v[...] = jnp.zeros_like(acc_v)

        def ffn_body(c, carry):
            xt = x_v[rows, :]
            for j in range(_FC // _FS):
                f0 = pl.multiple_of(c * _FC + j * _FS, _FS)
                cols = pl.ds(f0, _FS)
                gate = jnp.dot(xt, wg_v[:, cols], preferred_element_type=_F32)
                up = jnp.dot(xt, wu_v[:, cols], preferred_element_type=_F32)
                hid = (jnp.maximum(gate, 0.0) * up).astype(_BF16)
                acc_v[...] += jnp.dot(hid, wd_v[cols, :], preferred_element_type=_F32)
            return carry

        lax.fori_loop(0, F // _FC, ffn_body, 0)

        a = lax.dot_general(ot_v[:, rows], wo_v[...], (((0,), (0,)), ((), ())),
                            preferred_element_type=_F32)
        z = jnp.sum(x_v[rows, :].astype(_F32) * gw_v[...].astype(_F32), axis=-1, keepdims=True)
        g = jax.nn.sigmoid(z)
        out_ref[...] = (g * a + (1.0 - g) * acc_v[...]).astype(out_ref.dtype)

    scratch = [
        pltpu.VMEM((S, D), _BF16),
        pltpu.VMEM((D, H * Dh), _BF16),
        pltpu.VMEM((D, Dh), _BF16),
        pltpu.VMEM((D, Dh), _BF16),
        pltpu.VMEM((H * Dh, D), _BF16),
        pltpu.VMEM((D, F), _BF16),
        pltpu.VMEM((D, F), _BF16),
        pltpu.VMEM((F, D), _BF16),
        pltpu.VMEM((1, D), _BF16),
        pltpu.VMEM((H * Dh, S), _BF16),
        pltpu.VMEM((S, Dh), _BF16),
        pltpu.VMEM((Dh, S), _BF16),
        pltpu.VMEM((H * Dh, S), _BF16),
        pltpu.VMEM((_TM, D), _F32),
        pltpu.SemaphoreType.DMA((NX + 8,)),
    ] + [pltpu.VMEM((S, W), _F32)] * (2 * G) + [pltpu.VMEM((1, W), _F32)] * (2 * G)
    return kernel, scratch


@jax.jit
def pallas_gated_mix__grouped_kv_mqa__glu_gated_reglu__prompt_kernel(
    A_x: jax.Array,
    A_wq: jax.Array,
    A_wk: jax.Array,
    A_wv: jax.Array,
    A_wo: jax.Array,
    B_x: jax.Array,
    B_W_gate: jax.Array,
    B_W_up: jax.Array,
    B_W_down: jax.Array,
    gate_w: jax.Array,
):
    B, S, D = A_x.shape
    assert B == 1
    Dh = A_wk.shape[1]
    H = A_wq.shape[1] // Dh
    F = B_W_gate.shape[1]

    kernel, scratch = _make_kernel(S, D, H, Dh, F)
    any_spec = pl.BlockSpec(memory_space=pl.ANY)
    out = pl.pallas_call(
        kernel,
        grid=(S // _TM,),
        in_specs=[any_spec] * 9,
        out_specs=pl.BlockSpec((_TM, D), lambda i: (i, 0)),
        out_shape=jax.ShapeDtypeStruct((S, D), A_x.dtype),
        scratch_shapes=scratch,
        compiler_params=pltpu.CompilerParams(
            dimension_semantics=("arbitrary",),
            vmem_limit_bytes=110 * 1024 * 1024,
        ),
    )(A_x.reshape(S, D), A_wq, A_wk, A_wv, A_wo, B_W_gate, B_W_up, B_W_down,
      gate_w.reshape(1, D))
    return out.reshape(B, S, D)
```

```python
import contextlib
import math

import jax
import jax.numpy as jnp
from jax import lax
import jax.experimental.pallas as pl
import jax.experimental.pallas.tpu as pltpu

_F32 = jnp.float32
_BF16 = jnp.bfloat16

_TM = 256
_W = 512
_KC = 128
_G = 8
_FS = 256
_OR = 256
_OC = 128
_PROF = False


def _scope(name):
    return jax.named_scope(name) if _PROF else contextlib.nullcontext()


_NT = (((1,), (1,)), ((), ()))


def _tree(op, parts):
    cur = list(parts)
    while len(cur) > 1:
        nxt = [op(cur[2 * j], cur[2 * j + 1]) for j in range(len(cur) // 2)]
        if len(cur) % 2:
            nxt.append(cur[-1])
        cur = nxt
    return cur[0]


def _make_kernel(S, D, H, Dh, F):
    NQ = S // _W
    NB = H * NQ
    NC = S // _KC
    NT = S // _TM
    G = _G
    W = _W
    KC = _KC
    R = KC // 8
    HD = H * Dh
    q_scale = (Dh ** -0.5) * math.log2(math.e)
    x_pieces = [(0, 256), (256, 256), (512, 512), (1024, 512), (1536, 512)]
    QC = 256
    NQC = HD // QC

    def kernel(x_hbm, wq_hbm, wkt_hbm, wvt_hbm, wo_hbm, wg_hbm, wu_hbm, wd_hbm, gw_hbm,
               out_hbm,
               x_v, wq_v, wkvt_v, wo_v, wg_v, wu_v, wd_v, gw_v,
               qt_v, k_v, vt_v, ot_v, o_v, ga_v, g_v, hid_v, out_v,
               xsems, qsems, wsems, osems, *bufs):
        sbufs = bufs[:G]
        mbufs = bufs[G:]

        def x_copy(i):
            r0, n = x_pieces[i]
            return pltpu.make_async_copy(
                x_hbm.at[pl.ds(r0, n)], x_v.at[pl.ds(r0, n)], xsems.at[i])

        def wq_copy(j):
            return pltpu.make_async_copy(
                wq_hbm.at[:, pl.ds(j * QC, QC)], wq_v.at[:, pl.ds(j * QC, QC)], qsems.at[j])

        w_pairs = [(wkt_hbm, wkvt_v.at[pl.ds(0, Dh)]), (wvt_hbm, wkvt_v.at[pl.ds(Dh, Dh)]),
                   (gw_hbm, gw_v),
                   (wo_hbm, wo_v), (wg_hbm, wg_v), (wu_hbm, wu_v), (wd_hbm, wd_v)]

        def w_copy(j):
            return pltpu.make_async_copy(w_pairs[j][0], w_pairs[j][1], wsems.at[j])

        def out_copy(t):
            r0 = pl.multiple_of(t * _TM, _TM)
            return pltpu.make_async_copy(out_v.at[pl.ds(r0, _TM)], out_hbm.at[pl.ds(r0, _TM)], osems.at[t])

        def blk_idx(b):
            qi = b // H
            h = b % H
            if isinstance(b, int):
                return (slice(h * Dh, (h + 1) * Dh), slice(qi * W, (qi + 1) * W))
            return (pl.ds(pl.multiple_of(h * Dh, Dh), Dh), pl.ds(pl.multiple_of(qi * W, W), W))

        def attn_group(b_next0, b_cur0, fillers=()):
            do_qk = b_next0 is not None
            do_pv = b_cur0 is not None
            fillers = list(fillers)
            nfill = len(fillers)
            done = 0
            for g in range(G):
                sb = sbufs[g]
                mb = mbufs[g]
                if do_qk:
                    qt = qt_v[blk_idx(b_next0 + g)]
                    mx = None
                if do_pv:
                    m = jnp.broadcast_to(mb[...], (8, W))
                    acc = None
                    l = None
                for c in range(NC):
                    rows = slice(c * KC, (c + 1) * KC)
                    if do_pv:
                        sc = sb[rows, :].reshape(R, 8, W)
                    if do_qk:
                        s = jnp.dot(k_v[rows, :], qt, preferred_element_type=_F32)
                        sb[rows, :] = s
                        s3 = s.reshape(R, 8, W)
                        for r in range(R):
                            mx = s3[r] if mx is None else jnp.maximum(mx, s3[r])
                    while done * (G * NC) < nfill * (g * NC + c + 1) - (G * NC - 1) or (
                            done < nfill and done * (G * NC) <= nfill * (g * NC + c)):
                        fillers[done]()
                        done += 1
                    if do_pv:
                        p = jnp.exp2(sc - m[None])
                        t = _tree(jnp.add, [p[r] for r in range(R)])
                        l = t if l is None else l + t
                        pb = p.reshape(KC, W).astype(_BF16)
                        d = jnp.dot(vt_v[:, rows], pb, preferred_element_type=_F32)
                        acc = d if acc is None else acc + d
                if do_qk:
                    mb[...] = jnp.max(mx, axis=0, keepdims=True)
                if do_pv:
                    lt = jnp.sum(l, axis=0, keepdims=True)
                    ot_v[blk_idx(b_cur0 + g)] = (acc * (1.0 / lt)).astype(_BF16)
            while done < nfill:
                fillers[done]()
                done += 1

        with _scope("dmastart"):
            w_copy(0).start()
            w_copy(1).start()
            x_copy(0).start()
            wq_copy(0).start()
            wq_copy(1).start()

        def kv_proj(r0, n):
            rows = slice(r0, r0 + n)
            kvt = lax.dot_general(wkvt_v[...], x_v[rows, :], _NT, preferred_element_type=_F32)
            vt_v[:, rows] = kvt[Dh:, :].astype(_BF16)
            k_v[rows, :] = kvt[:Dh, :].T.astype(_BF16)

        def q_proj(r0, n, c0, nc):
            rows = slice(r0, r0 + n)
            cols = slice(c0, c0 + nc)
            q = jnp.dot(x_v[rows, :], wq_v[:, cols], preferred_element_type=_F32) * q_scale
            qt_v[cols, rows] = q.T.astype(_BF16)

        with _scope("wwait"):
            w_copy(0).wait()
            w_copy(1).wait()
            x_copy(0).wait()
            x_copy(1).start()
            wq_copy(0).wait()
            wq_copy(2).start()
        with _scope("proj"):
            kv_proj(0, 256)
            q_proj(0, 256, 0, QC)
            with _scope("w1"):
                wq_copy(1).wait()
            wq_copy(3).start()
            q_proj(0, 256, QC, QC)
            with _scope("w2"):
                x_copy(1).wait()
            x_copy(2).start()
            kv_proj(256, 256)
            q_proj(256, 256, 0, 2 * QC)
            with _scope("w3"):
                wq_copy(2).wait()
                wq_copy(3).wait()
            x_copy(3).start()
            x_copy(4).start()
            q_proj(0, 512, 2 * QC, 2 * QC)
            with _scope("w4"):
                x_copy(2).wait()
            kv_proj(512, 512)
            q_proj(512, 512, 0, HD)
            with _scope("w5"):
                x_copy(3).wait()
                x_copy(4).wait()
            for j in range(2, len(w_pairs)):
                w_copy(j).start()
            for r0 in (1024, 1536):
                kv_proj(r0, 512)
                q_proj(r0, 512, 0, HD)

        with _scope("qk0"):
            attn_group(0, None)

        def body(i, carry):
            attn_group((i + 1) * G, i * G)
            return carry

        n_it = NB // G
        with _scope("attnloop"):
            lax.fori_loop(0, n_it - 1, body, 0)

        for j in range(2, len(w_pairs)):
            w_copy(j).wait()

        def prep_rows(r0):
            def f():
                rows = slice(r0, r0 + _OR)
                o_v[rows, :] = ot_v[:, rows].T
                gw = gw_v[...].astype(_F32)
                z = _tree(jnp.add, [
                    x_v[rows, r * 128:(r + 1) * 128].astype(_F32) * gw[r:r + 1, :]
                    for r in range(D // 128)])
                z = jnp.sum(z, axis=-1, keepdims=True)
                g_v[rows, :] = jax.nn.sigmoid(z)
            return f

        def oproj_piece(r0, c0):
            def f():
                rows = slice(r0, r0 + _OR)
                cols = slice(c0, c0 + _OC)
                a = jnp.dot(o_v[rows, :], wo_v[:, cols], preferred_element_type=_F32)
                ga_v[rows, cols] = g_v[rows, :] * a
            return f

        def oproj_rows(r0):
            pieces = [oproj_piece(r0, c0) for c0 in range(0, D, _OC)]

            def first():
                prep_rows(r0)()
                pieces[0]()
            return [first] + pieces[1:]

        with _scope("pvlast_oproj"):
            done_rows = S - _W
            fill = []
            for r0 in range(0, done_rows, _OR):
                fill.extend(oproj_rows(r0))
            attn_group(None, (n_it - 1) * G, fill)
            for r0 in range(done_rows, S, _OR):
                for f in oproj_rows(r0):
                    f()

        def tile_body(t, carry):
            r0 = pl.multiple_of(t * _TM, _TM)
            rows = pl.ds(r0, _TM)
            with _scope("ffn"):
                xt = x_v[rows, :]
                for j in range(F // _FS):
                    cols = slice(j * _FS, (j + 1) * _FS)
                    gate = jnp.dot(xt, wg_v[:, cols], preferred_element_type=_F32)
                    up = jnp.dot(xt, wu_v[:, cols], preferred_element_type=_F32)
                    hid_v[:, cols] = (jnp.maximum(gate, 0.0) * up).astype(_BF16)
                b = jnp.dot(hid_v[...], wd_v[...], preferred_element_type=_F32)
                out_v[rows, :] = (ga_v[rows, :] + (1.0 - g_v[rows, :]) * b).astype(out_v.dtype)
            out_copy(t).start()
            return carry

        lax.fori_loop(0, NT, tile_body, 0)
        for t in range(NT):
            out_copy(t).wait()

    scratch = [
        pltpu.VMEM((S, D), _BF16),
        pltpu.VMEM((D, HD), _BF16),
        pltpu.VMEM((2 * Dh, D), _BF16),
        pltpu.VMEM((HD, D), _BF16),
        pltpu.VMEM((D, F), _BF16),
        pltpu.VMEM((D, F), _BF16),
        pltpu.VMEM((F, D), _BF16),
        pltpu.VMEM((D // 128, 128), _BF16),
        pltpu.VMEM((HD, S), _BF16),
        pltpu.VMEM((S, Dh), _BF16),
        pltpu.VMEM((Dh, S), _BF16),
        pltpu.VMEM((HD, S), _BF16),
        pltpu.VMEM((S, HD), _BF16),
        pltpu.VMEM((S, D), _F32),
        pltpu.VMEM((S, 1), _F32),
        pltpu.VMEM((_TM, F), _BF16),
        pltpu.VMEM((S, D), _BF16),
        pltpu.SemaphoreType.DMA((len(x_pieces),)),
        pltpu.SemaphoreType.DMA((NQC,)),
        pltpu.SemaphoreType.DMA((7,)),
        pltpu.SemaphoreType.DMA((NT,)),
    ] + [pltpu.VMEM((S, W), _F32)] * G + [pltpu.VMEM((1, W), _F32)] * G
    return kernel, scratch


@jax.jit
def pallas_gated_mix__grouped_kv_mqa__glu_gated_reglu__prompt_kernel(
    A_x: jax.Array,
    A_wq: jax.Array,
    A_wk: jax.Array,
    A_wv: jax.Array,
    A_wo: jax.Array,
    B_x: jax.Array,
    B_W_gate: jax.Array,
    B_W_up: jax.Array,
    B_W_down: jax.Array,
    gate_w: jax.Array,
):
    B, S, D = A_x.shape
    assert B == 1
    Dh = A_wk.shape[1]
    H = A_wq.shape[1] // Dh
    F = B_W_gate.shape[1]

    kernel, scratch = _make_kernel(S, D, H, Dh, F)
    any_spec = pl.BlockSpec(memory_space=pl.ANY)
    out = pl.pallas_call(
        kernel,
        in_specs=[any_spec] * 9,
        out_specs=any_spec,
        out_shape=jax.ShapeDtypeStruct((S, D), A_x.dtype),
        scratch_shapes=scratch,
        compiler_params=pltpu.CompilerParams(
            vmem_limit_bytes=120 * 1024 * 1024,
        ),
    )(A_x.reshape(S, D), A_wq, A_wk.T, A_wv.T, A_wo, B_W_gate, B_W_up, B_W_down,
      gate_w.reshape(D // 128, 128))
    return out.reshape(B, S, D)
```

```python
import contextlib
import math

import jax
import jax.numpy as jnp
from jax import lax
import jax.experimental.pallas as pl
import jax.experimental.pallas.tpu as pltpu

_F32 = jnp.float32
_BF16 = jnp.bfloat16
_U32 = jnp.uint32

_TM = 128
_W = 512
_KC = 128
_G = 4
_FS = 256
_OR = 256
_OC = 128
_KBS = (16, 24, 16, 16, 24, 16, 16, 24, 16, 24)
_PROF = False
_PVLAG = 1
_LAST = 128
_HOLD = 4
_PVLAG_E = 0


def _scope(name):
    return jax.named_scope(name) if _PROF else contextlib.nullcontext()


_NT = (((1,), (1,)), ((), ()))


def _tree(op, parts):
    cur = list(parts)
    while len(cur) > 1:
        nxt = [op(cur[2 * j], cur[2 * j + 1]) for j in range(len(cur) // 2)]
        if len(cur) % 2:
            nxt.append(cur[-1])
        cur = nxt
    return cur[0]


def _make_kernel(S, D, H, Dh, F):
    W, KC, G, TM = _W, _KC, _G, _TM
    NQ = S // W
    NB = H * NQ
    NC = S // KC
    R = KC // 8
    LT = W // 128
    HD = H * Dh
    NV = sum(_KBS)
    SM = S - NV
    NF = S // TM
    NG = NB // G
    GF = NG // NF
    BF = G
    FP = F // GF
    NJ = F // _FS // GF
    assert NV % 16 == 0 and H % G == 0 and NG % NF == 0 and F % (_FS * GF) == 0
    kb_offs = [sum(_KBS[:t]) for t in range(len(_KBS))]
    n_small = (NC * KC - SM) // 16
    assert n_small <= NC
    qk_rows = [KC - 16] * n_small + [KC] * (NC - n_small)
    qk_start = [sum(qk_rows[:c]) for c in range(NC)]
    q_scale = (Dh ** -0.5) * math.log2(math.e)
    x_pieces = [(0, 256), (256, 256), (512, 512), (1024, 512), (1536, 512)]
    QC = 256
    NQC = HD // QC
    out_pieces = [(0, S - W), (S - W, W - _LAST), (S - _LAST, _LAST)]
    GR = 16
    V0 = Dh + GR

    def kernel(x_hbm, wq_hbm, wkt_hbm, wvt_hbm, wo_hbm, wg_hbm, wu_hbm, wd_hbm, gw_hbm,
               out_hbm,
               x_u, wq_u, wkvt_u, wo_u, wg_u, wu_u, wd_u, gw_v,
               qt_u, k_u, vt_u, ot_u, o_u, out_u,
               kb_v, sv_v, vm_v, b_v, g_v, qf_v, bs_v,
               xsems, qsems, wsems, osems, *bufs):
        sbufs = bufs[:G]
        mbufs = bufs[G:]
        x_v, wq_v, wkvt_v, wo_v, wg_v, wu_v, wd_v, qt_v, vt_v, ot_v, o_v, out_v = [
            r.bitcast(_BF16) for r in
            (x_u, wq_u, wkvt_u, wo_u, wg_u, wu_u, wd_u, qt_u, vt_u, ot_u, o_u, out_u)]

        def x_copy(i):
            r0, n = x_pieces[i]
            return pltpu.make_async_copy(
                x_hbm.at[pl.ds(r0, n)], x_v.at[pl.ds(r0, n)], xsems.at[i])

        def wq_copy(j):
            return pltpu.make_async_copy(
                wq_hbm.at[:, pl.ds(j * QC, QC)], wq_v.at[:, pl.ds(j * QC, QC)], qsems.at[j])

        w_pairs = [(wkt_hbm, wkvt_v.at[pl.ds(0, Dh)]), (wvt_hbm, wkvt_v.at[pl.ds(V0, Dh)]),
                   (gw_hbm, gw_v)]
        for part in range(GF):
            fc = pl.ds(part * FP, FP)
            w_pairs += [(wg_hbm.at[:, fc], wg_v.at[part]), (wu_hbm.at[:, fc], wu_v.at[part]),
                        (wd_hbm.at[fc], wd_v.at[part])]
        w_pairs.append((wo_hbm, wo_v))

        def w_copy(j):
            return pltpu.make_async_copy(w_pairs[j][0], w_pairs[j][1], wsems.at[j])

        def out_copy(t):
            r0, n = out_pieces[t]
            return pltpu.make_async_copy(out_v.at[pl.ds(r0, n)], out_hbm.at[pl.ds(r0, n)], osems.at[t])

        def attn_group(b_next0, b_cur0, fillers=()):
            do_qk = b_next0 is not None
            do_pv = b_cur0 is not None
            fillers = list(fillers)
            nfill = len(fillers)
            done = 0
            st = dict(mx=None, qt=None, m=None, acc=None, l=None)

            def load_scores(g, c):
                lo, hi = c * KC, (c + 1) * KC
                parts = []
                if lo < SM:
                    parts.append(sbufs[g][lo:min(hi, SM), :])
                if hi > SM:
                    parts.append(sv_v[g, max(lo, SM) - SM:hi - SM, :])
                sc = parts[0] if len(parts) == 1 else jnp.concatenate(parts, axis=0)
                if c == 0:
                    m = jnp.max(jnp.maximum(mbufs[g][...], vm_v[g]), axis=0, keepdims=True)
                    st["m"] = jnp.broadcast_to(m, (8, W))
                return sc.reshape(R, 8, W), st["m"]

            def qk(g, c):
                if c == 0:
                    st["qt"] = qt_v[b_next0 + g]
                    st["mx"] = None
                r0, n = qk_start[c], qk_rows[c]
                kc = pltpu.bitcast(k_u[r0 // 2:(r0 + n) // 2, :], _BF16)
                s = jnp.dot(kc, st["qt"], preferred_element_type=_F32)
                sbufs[g][r0:r0 + n, :] = s
                s3 = s.reshape(n // 8, 8, W)
                for r in range(n // 8):
                    st["mx"] = s3[r] if st["mx"] is None else jnp.maximum(st["mx"], s3[r])
                if c == NC - 1:
                    mbufs[g][...] = st["mx"]

            def pv(g, c, sc, m):
                lo, hi = c * KC, (c + 1) * KC
                p = jnp.exp2(sc - m[None])
                t = _tree(jnp.add, [p[r] for r in range(R)])
                st["l"] = t if c == 0 else st["l"] + t
                pb = p.reshape(KC, W).astype(_BF16)
                d = jnp.dot(vt_v[:, lo:hi], pb, preferred_element_type=_F32)
                st["acc"] = d if c == 0 else st["acc"] + d
                if c == NC - 1:
                    lt = jnp.sum(st["l"], axis=0, keepdims=True)
                    ot_v[b_cur0 + g] = (st["acc"] * (1.0 / lt)).astype(_BF16)

            steps = [(g, c) for g in range(G) for c in range(NC)]
            pend = []
            for n, (g, c) in enumerate(steps):
                if do_pv:
                    pend.append((g, c) + load_scores(g, c))
                if do_qk:
                    qk(g, c)
                while done < nfill and done * len(steps) <= nfill * n:
                    fillers[done]()
                    done += 1
                if len(pend) > (_PVLAG if do_qk else _PVLAG_E):
                    pv(*pend.pop(0))
            while pend:
                pv(*pend.pop(0))
            while done < nfill:
                fillers[done]()
                done += 1
            return st["l"][:, :128] if do_pv else None

        with _scope("dmastart"):
            x_copy(0).start()
            wq_copy(0).start()
            wq_copy(1).start()
            for j in range(3):
                w_copy(j).start()

        def kv_proj(r0, n):
            rows = slice(r0, r0 + n)
            kvt = lax.dot_general(wkvt_v[...], x_v[rows, :], _NT, preferred_element_type=_F32)
            vt_v[:, rows] = kvt[V0:, :].astype(_BF16)
            kg = jnp.concatenate([kvt[:Dh, :], jax.nn.sigmoid(kvt[Dh:Dh + 8, :])], axis=0).T
            k_u[r0 // 2:(r0 + n) // 2, :] = pltpu.bitcast(kg[:, :Dh].astype(_BF16), _U32)
            g_v[rows, :] = kg[:, Dh:Dh + 1]

        def q_proj(r0, n, c0, nc):
            rows = slice(r0, r0 + n)
            cols = slice(c0, c0 + nc)
            q = jnp.dot(x_v[rows, :], wq_v[:, cols], preferred_element_type=_F32) * q_scale
            qtb = q.T.astype(_BF16)
            qtf = qtb.astype(_F32)
            lanes = slice(r0 % W, r0 % W + n)
            for h in range(c0 // Dh, (c0 + nc) // Dh):
                hr = slice(h * Dh - c0, (h + 1) * Dh - c0)
                qt_v[(r0 // W) * H + h, :, lanes] = qtb[hr, :]
                qf_v[(r0 // W) * H + h, :, lanes] = qtf[hr, :]

        with _scope("wwait"):
            x_copy(0).wait()
            x_copy(1).start()
            wq_copy(0).wait()
            wq_copy(2).start()
        with _scope("proj"):
            q_proj(0, 256, 0, QC)
            wq_copy(1).wait()
            for j in range(3):
                w_copy(j).wait()
            wq_copy(3).start()
            gw = gw_v[...].astype(_F32)
            first_row = lax.broadcasted_iota(jnp.int32, (GR, 128), 0) == 0
            for c in range(D // 128):
                tile = jnp.where(first_row, jnp.broadcast_to(gw[c:c + 1, :], (GR, 128)), 0.0)
                wkvt_v[Dh:V0, c * 128:(c + 1) * 128] = tile.astype(_BF16)
            q_proj(0, 256, QC, QC)
            x_copy(1).wait()
            x_copy(2).start()
            kv_proj(0, 512)
            q_proj(256, 256, 0, 2 * QC)
            wq_copy(2).wait()
            wq_copy(3).wait()
            x_copy(3).start()
            x_copy(4).start()
            q_proj(0, 512, 2 * QC, 2 * QC)
            x_copy(2).wait()
            for j in range(3, len(w_pairs)):
                w_copy(j).start()
            kv_proj(512, 512)
            q_proj(512, 512, 0, HD)
            x_copy(3).wait()
            x_copy(4).wait()
            kv_proj(1024, 512)
            kv_proj(1536, 512)
            for r0 in (1024, 1536):
                q_proj(r0, 512, 0, HD)
            kf = pltpu.bitcast(k_u[SM // 2:, :], _BF16).astype(_F32)
            for d in range(Dh):
                kb_v[d] = jnp.broadcast_to(kf[:, d:d + 1], (NV, 128))

        with _scope("qk0"):
            attn_group(0, None)
            kc = pltpu.bitcast(k_u[SM // 2:, :], _BF16)
            for g in range(BF):
                s = jnp.dot(kc, qt_v[g], preferred_element_type=_F32)
                sv_v[g] = s
                s3 = s.reshape(NV // 8, 8, W)
                vm_v[g] = _tree(jnp.maximum, [s3[r] for r in range(NV // 8)])

        def zero_of(v):
            return jnp.minimum(jnp.maximum(v, 0.0), 0.0)

        def vpu_piece(b, slot, kk, kb, j, z):
            qblk = qf_v[b, :, j * 128:(j + 1) * 128]
            acc = None
            for d in range(Dh):
                qb = jnp.broadcast_to(qblk[d:d + 1, :], (8, 128))
                t = kb_v[d, kk:kk + kb, :].reshape(kb // 8, 8, 128) * qb[None]
                if acc is None:
                    acc = t if z is None else t + z[None]
                else:
                    acc = acc + t
            sv_v[slot, kk:kk + kb, j * 128:(j + 1) * 128] = acc.reshape(kb, 128)
            return _tree(jnp.maximum, [acc[r] for r in range(kb // 8)]), acc[0]

        def ffn_part(q, grp, start):
            i = q // GF
            part = q % GF
            rows = pl.ds(pl.multiple_of(i * TM, TM), TM)
            pieces = [(e, kk, kb, j) for e in range(G) for j in range(LT)
                      for kk, kb in zip(kb_offs, _KBS)]
            items = []
            for j in range(NJ + 1):
                if j < NJ:
                    items.append(("gu", j, 2))
                if j >= 1:
                    items.append(("d", j - 1, 1))
            total = sum(it[2] for it in items)
            accum = 0
            done = 0
            last = start
            mv = None
            hid = {}
            xt = x_v[rows, :]
            for kind, j, cost in items:
                cols = slice(j * _FS, (j + 1) * _FS)
                if kind == "gu":
                    gate = jnp.dot(xt, wg_v[part, :, cols], preferred_element_type=_F32)
                    up = jnp.dot(xt, wu_v[part, :, cols], preferred_element_type=_F32)
                    hid[j] = (jnp.maximum(gate, 0.0) * up).astype(_BF16)
                else:
                    dv = jnp.dot(hid.pop(j), wd_v[part, cols, :], preferred_element_type=_F32)
                    if j == 0:
                        bs_v[...] = jnp.where(part == 0, 0.0, bs_v[...]) + dv
                    elif j == NJ - 1:
                        tot = bs_v[...] + dv
                        bs_v[...] = tot
                        b_v[rows, :] = tot
                    else:
                        bs_v[...] += dv
                accum += cost
                tgt = min(len(pieces), (len(pieces) * accum + total - 1) // total)
                while done < tgt:
                    e, kk, kb, jj = pieces[done]
                    z = zero_of(last) if last is not None else None
                    mxv, last = vpu_piece(grp * G + e, e, kk, kb, jj, z)
                    mv = mxv if kk == 0 else jnp.maximum(mv, mxv)
                    if kk + kb == NV:
                        vm_v[e, :, jj * 128:(jj + 1) * 128] = mv
                    done += 1

        for j in range(3, 6):
            w_copy(j).wait()
        bs_v[...] = jnp.zeros_like(bs_v)

        def main_body(q, carry):
            for part in range(1, GF):
                @pl.when(q == part)
                def _():
                    for j in range(3 + 3 * part, 6 + 3 * part):
                        w_copy(j).wait()

            late = attn_group((q + 1) * G, q * G)
            ffn_part(q, q + 1, late)
            return carry

        with _scope("mainloop"):
            lax.fori_loop(0, NG - 1, main_body, 0)

        w_copy(len(w_pairs) - 1).wait()

        def transpose_o(r0, n):
            lanes = slice(r0 % W, r0 % W + n)
            ot = jnp.concatenate(
                [ot_v[(r0 // W) * H + h, :, lanes] for h in range(H)], axis=0)
            o_v[r0:r0 + n, :] = ot.T

        def oproj_piece(r0, n, c0, nc, prep):
            def f():
                rows = slice(r0, r0 + n)
                cols = slice(c0, c0 + nc)
                if prep:
                    transpose_o(r0, n)
                a = jnp.dot(o_v[rows, :], wo_v[:, cols], preferred_element_type=_F32)
                g = g_v[rows, :]
                out_v[rows, cols] = (g * a + (1.0 - g) * b_v[rows, cols]).astype(_BF16)
            return f

        def oproj_rows(lo, hi, prep):
            fs = []
            r0 = lo
            while r0 < hi:
                n = min(_OR, hi - r0)
                nc = _OC * _OR // n
                fs += [oproj_piece(r0, n, c0, nc, prep and c0 == 0) for c0 in range(0, D, nc)]
                r0 += n
            return fs

        def last_ffn_items():
            i = NF - 1
            rows = slice(i * TM, (i + 1) * TM)
            hid = {}
            fs = []

            def gate(j):
                def f():
                    cols = slice(j * _FS, (j + 1) * _FS)
                    hid[j] = jnp.dot(x_v[rows, :], wg_v[GF - 1, :, cols], preferred_element_type=_F32)
                return f

            def up(j):
                def f():
                    cols = slice(j * _FS, (j + 1) * _FS)
                    u = jnp.dot(x_v[rows, :], wu_v[GF - 1, :, cols], preferred_element_type=_F32)
                    hid[j] = (jnp.maximum(hid[j], 0.0) * u).astype(_BF16)
                return f

            def dn(j):
                def f():
                    cols = slice(j * _FS, (j + 1) * _FS)
                    dv = jnp.dot(hid.pop(j), wd_v[GF - 1, cols, :], preferred_element_type=_F32)
                    b_v[rows, :] += dv
                return f

            for j in range(NJ + 1):
                if j < NJ:
                    fs += [gate(j), up(j)]
                if j >= 1:
                    fs.append(dn(j - 1))
            return fs

        with _scope("pvlast_oproj"):
            fill = last_ffn_items() + oproj_rows(0, S - W, True)
            attn_group(None, NB - G, fill[:len(fill) - _HOLD])
            for r0 in range(S - W, S, _OR):
                transpose_o(r0, _OR)
            for f in fill[len(fill) - _HOLD:]:
                f()
            out_copy(0).start()
            for t in range(1, len(out_pieces)):
                r0, n = out_pieces[t]
                for f in oproj_rows(r0, r0 + n, False):
                    f()
                out_copy(t).start()
        for t in range(len(out_pieces)):
            out_copy(t).wait()

    scratch = [
        pltpu.VMEM((S // 2, D), _U32),
        pltpu.VMEM((D // 2, HD), _U32),
        pltpu.VMEM(((V0 + Dh) // 2, D), _U32),
        pltpu.VMEM((HD // 2, D), _U32),
        pltpu.VMEM((GF, D // 2, FP), _U32),
        pltpu.VMEM((GF, D // 2, FP), _U32),
        pltpu.VMEM((GF, FP // 2, D), _U32),
        pltpu.VMEM((D // 128, 128), _BF16),
        pltpu.VMEM((NB, Dh // 2, W), _U32),
        pltpu.VMEM((S // 2, Dh), _U32),
        pltpu.VMEM((Dh // 2, S), _U32),
        pltpu.VMEM((NB, Dh // 2, W), _U32),
        pltpu.VMEM((S // 2, HD), _U32),
        pltpu.VMEM((S // 2, D), _U32),
        pltpu.VMEM((Dh, NV, 128), _F32),
        pltpu.VMEM((BF, NV, W), _F32),
        pltpu.VMEM((BF, 8, W), _F32),
        pltpu.VMEM((S, D), _F32),
        pltpu.VMEM((S, 1), _F32),
        pltpu.VMEM((NB, Dh, W), _F32),
        pltpu.VMEM((TM, D), _F32),
        pltpu.SemaphoreType.DMA((len(x_pieces),)),
        pltpu.SemaphoreType.DMA((NQC,)),
        pltpu.SemaphoreType.DMA((4 + 3 * GF,)),
        pltpu.SemaphoreType.DMA((len(out_pieces),)),
    ] + [pltpu.VMEM((SM, W), _F32)] * G + [pltpu.VMEM((8, W), _F32)] * G
    return kernel, scratch


@jax.jit
def pallas_gated_mix__grouped_kv_mqa__glu_gated_reglu__prompt_kernel(
    A_x: jax.Array,
    A_wq: jax.Array,
    A_wk: jax.Array,
    A_wv: jax.Array,
    A_wo: jax.Array,
    B_x: jax.Array,
    B_W_gate: jax.Array,
    B_W_up: jax.Array,
    B_W_down: jax.Array,
    gate_w: jax.Array,
):
    B, S, D = A_x.shape
    assert B == 1
    Dh = A_wk.shape[1]
    H = A_wq.shape[1] // Dh
    F = B_W_gate.shape[1]

    kernel, scratch = _make_kernel(S, D, H, Dh, F)
    any_spec = pl.BlockSpec(memory_space=pl.ANY)
    out = pl.pallas_call(
        kernel,
        in_specs=[any_spec] * 9,
        out_specs=any_spec,
        out_shape=jax.ShapeDtypeStruct((S, D), A_x.dtype),
        scratch_shapes=scratch,
        compiler_params=pltpu.CompilerParams(
            vmem_limit_bytes=120 * 1024 * 1024,
        ),
    )(A_x.reshape(S, D), A_wq, A_wk.T, A_wv.T, A_wo, B_W_gate, B_W_up, B_W_down,
      gate_w.reshape(D // 128, 128))
    return out.reshape(B, S, D)
```

```python
import math

import jax
import jax.numpy as jnp
from jax import lax
import jax.experimental.pallas as pl
import jax.experimental.pallas.tpu as pltpu

_F32 = jnp.float32
_BF16 = jnp.bfloat16
_U32 = jnp.uint32

_TM = 128
_W = 512
_KC = 128
_G = 4
_FS = 256
_OR = 256
_OC = 128
_NV = 224
_SA = (0, 0, 2, 1, 2, 2, 1, 1, 2, 1, 2, 1, 1, 0, 0, 0)
_PF = (2, 2, 3, 2, 3)
_DUE = 3
_C0 = 2
_LAST = 128
_HOLD = 4

_NT = (((1,), (1,)), ((), ()))


def _tree(op, parts):
    cur = list(parts)
    while len(cur) > 1:
        nxt = [op(cur[2 * j], cur[2 * j + 1]) for j in range(len(cur) // 2)]
        if len(cur) % 2:
            nxt.append(cur[-1])
        cur = nxt
    return cur[0]


def _zero_of(v):
    return jnp.minimum(jnp.maximum(v, 0.0), 0.0)


def _make_kernel(S, D, H, Dh, F):
    W, KC, G, TM, NV = _W, _KC, _G, _TM, _NV
    NB = H * (S // W)
    NC = S // KC
    R = KC // 8
    LT = W // 128
    HD = H * Dh
    SM = S - NV
    NF = S // TM
    NG = NB // G
    GF = NG // NF
    FP = F // GF
    NJ = FP // _FS
    assert NV % 16 == 0 and H % G == 0 and NG % NF == 0 and F % (_FS * GF) == 0
    assert len(_SA) == NC and S == 2048 and W == 512 and HD % 1024 == 0

    a_steps = [n for n in range(1, G * NC) if _SA[n % NC]]
    NA = len(a_steps)
    pieces = []
    for e in range(G):
        for j in range(LT):
            kk = 0
            while kk < NV:
                n = len(pieces)
                size = _SA[a_steps[n] % NC] if n < NA else _PF[(n - NA) % len(_PF)]
                kb = min(8 * size, NV - kk)
                pieces.append((e, kk, kb, j))
                kk += kb
    assert all(p[0] == 0 for p in pieces[:NA])

    n_big = NC - NV // 16
    assert n_big >= 0
    big = set((NC * t) // n_big for t in range(n_big))
    qk_rows = [KC if c in big else KC - 16 for c in range(NC)]
    qk_start = [sum(qk_rows[:c]) for c in range(NC)]
    q_scale = (Dh ** -0.5) * math.log2(math.e)
    x_pieces = [(0, 256), (256, 256), (512, 512), (1024, 512), (1536, 512)]
    QC = HD // 4
    out_pieces = [(0, S - W), (S - W, W - _LAST), (S - _LAST, _LAST)]
    GR = 16
    V0 = Dh + GR

    def kernel(x_hbm, wq_hbm, wkt_hbm, wvt_hbm, wo_hbm, wg_hbm, wu_hbm, wd_hbm, gw_hbm,
               out_hbm,
               x_u, wq_u, wkvt_u, wo_u, wg_u, wu_u, wd_u, gw_v,
               qt_u, k_u, vt_u, ot_u, o_u, out_u,
               kb_v, sv_v, vm_v, b_v, g_v, qf_v, bs_v,
               xsems, qsems, wsems, osems, *bufs):
        sbufs = bufs[:G]
        mbufs = bufs[G:]
        x_v, wq_v, wkvt_v, wo_v, wg_v, wu_v, wd_v, qt_v, vt_v, ot_v, o_v, out_v = [
            r.bitcast(_BF16) for r in
            (x_u, wq_u, wkvt_u, wo_u, wg_u, wu_u, wd_u, qt_u, vt_u, ot_u, o_u, out_u)]

        def x_copy(i):
            r0, n = x_pieces[i]
            return pltpu.make_async_copy(
                x_hbm.at[pl.ds(r0, n)], x_v.at[pl.ds(r0, n)], xsems.at[i])

        def wq_copy(j):
            return pltpu.make_async_copy(
                wq_hbm.at[:, pl.ds(j * QC, QC)], wq_v.at[:, pl.ds(j * QC, QC)], qsems.at[j])

        w_pairs = [(wkt_hbm, wkvt_v.at[pl.ds(0, Dh)]), (wvt_hbm, wkvt_v.at[pl.ds(V0, Dh)]),
                   (gw_hbm, gw_v)]
        for part in range(GF):
            fc = pl.ds(part * FP, FP)
            w_pairs += [(wg_hbm.at[:, fc], wg_v.at[part]), (wu_hbm.at[:, fc], wu_v.at[part]),
                        (wd_hbm.at[fc], wd_v.at[part])]
        w_pairs.append((wo_hbm, wo_v))

        def w_copy(j):
            return pltpu.make_async_copy(w_pairs[j][0], w_pairs[j][1], wsems.at[j])

        def out_copy(t):
            r0, n = out_pieces[t]
            return pltpu.make_async_copy(
                out_v.at[pl.ds(r0, n)], out_hbm.at[pl.ds(r0, n)], osems.at[t])

        def vpu_piece(b, slot, kk, kb, j, z):
            qblk = qf_v[b, :, j * 128:(j + 1) * 128]
            acc = None
            for d in range(Dh):
                qb = jnp.broadcast_to(qblk[d:d + 1, :], (8, 128))
                t = kb_v[d, kk:kk + kb, :].reshape(kb // 8, 8, 128) * qb[None]
                acc = t + z[None] if acc is None else acc + t
            sv_v[slot, kk:kk + kb, j * 128:(j + 1) * 128] = acc.reshape(kb, 128)
            return _tree(jnp.maximum, [acc[r] for r in range(kb // 8)]), acc[0]

        def make_chain(grp):
            cs = dict(last=None, mv=None, done=0)

            def emit(upto):
                while cs["done"] < min(upto, len(pieces)):
                    e, kk, kb, j = pieces[cs["done"]]
                    slot = G if e == 0 else e
                    mxv, cs["last"] = vpu_piece(grp * G + e, slot, kk, kb, j, _zero_of(cs["last"]))
                    cs["mv"] = mxv if kk == 0 else jnp.maximum(cs["mv"], mxv)
                    if kk + kb == NV:
                        vm_v[slot, :, j * 128:(j + 1) * 128] = cs["mv"]
                    cs["done"] += 1
            return cs, emit

        def attn_group(b_next0, b_cur0, fillers=(), chain=None):
            do_qk = b_next0 is not None
            do_pv = b_cur0 is not None
            fillers = list(fillers)
            nfill = len(fillers)
            done = 0
            st = dict(mx=None, qt=None, m=None, acc=None, l=None)
            taps = []

            def load_scores(g, c):
                lo, hi = c * KC, (c + 1) * KC
                parts = []
                if lo < SM:
                    parts.append(sbufs[g][lo:min(hi, SM), :])
                if hi > SM:
                    parts.append(sv_v[g, max(lo, SM) - SM:hi - SM, :])
                sc = parts[0] if len(parts) == 1 else jnp.concatenate(parts, axis=0)
                if c == 0:
                    m = jnp.max(jnp.maximum(mbufs[g][...], vm_v[g]), axis=0, keepdims=True)
                    st["m"] = jnp.broadcast_to(m, (8, W))
                return sc.reshape(R, 8, W), st["m"]

            def qk(g, c):
                if c == 0:
                    st["qt"] = qt_v[b_next0 + g]
                    st["mx"] = None
                r0, n = qk_start[c], qk_rows[c]
                kc = pltpu.bitcast(k_u[r0 // 2:(r0 + n) // 2, :], _BF16)
                s = jnp.dot(kc, st["qt"], preferred_element_type=_F32)
                sbufs[g][r0:r0 + n, :] = s
                s3 = s.reshape(n // 8, 8, W)
                for r in range(n // 8):
                    st["mx"] = s3[r] if st["mx"] is None else jnp.maximum(st["mx"], s3[r])
                if c == NC - 1:
                    mbufs[g][...] = st["mx"]

            def pv(g, c, sc, m):
                lo, hi = c * KC, (c + 1) * KC
                if chain is not None:
                    ready = [v for (due, v) in taps if due <= g * NC + c]
                    taps[:] = [t for t in taps if t[0] > g * NC + c]
                    if c >= _C0:
                        link = st["l"]
                        if ready:
                            head = _tree(jnp.add, [link[:, :128]] + ready)
                            link = jnp.concatenate([head, link[:, 128:]], axis=1)
                        m = m + _zero_of(link)
                    elif ready:
                        head = m[:, :128] + _zero_of(_tree(jnp.add, ready))
                        m = jnp.concatenate([head, m[:, 128:]], axis=1)
                p = jnp.exp2(sc - m[None])
                t = _tree(jnp.add, [p[r] for r in range(R)])
                st["l"] = t if c == 0 else st["l"] + t
                pb = p.reshape(KC, W).astype(_BF16)
                d = jnp.dot(vt_v[:, lo:hi], pb, preferred_element_type=_F32)
                st["acc"] = d if c == 0 else st["acc"] + d
                if c == NC - 1:
                    lt = jnp.sum(st["l"], axis=0, keepdims=True)
                    ot_v[b_cur0 + g] = (st["acc"] * (1.0 / lt)).astype(_BF16)

            steps = [(g, c) for g in range(G) for c in range(NC)]
            pend = []
            for n, (g, c) in enumerate(steps):
                if do_pv:
                    pend.append((g, c) + load_scores(g, c))
                if do_qk:
                    qk(g, c)
                while done < nfill and done * len(steps) <= nfill * n:
                    fillers[done]()
                    done += 1
                if len(pend) > (1 if do_qk else 0):
                    pv(*pend.pop(0))
                if chain is not None and n in a_steps:
                    chain[0]["last"] = st["l"][:, :128]
                    chain[1](chain[0]["done"] + 1)
                    taps.append((n + _DUE, chain[0]["last"]))
            while pend:
                pv(*pend.pop(0))
            if chain is not None:
                chain[0]["last"] = st["l"][:, :128]
            while done < nfill:
                fillers[done]()
                done += 1

        def kv_proj(r0, n):
            rows = slice(r0, r0 + n)
            kvt = lax.dot_general(wkvt_v[...], x_v[rows, :], _NT, preferred_element_type=_F32)
            vt_v[:, rows] = kvt[V0:, :].astype(_BF16)
            kg = jnp.concatenate([kvt[:Dh, :], jax.nn.sigmoid(kvt[Dh:Dh + 8, :])], axis=0).T
            k_u[r0 // 2:(r0 + n) // 2, :] = pltpu.bitcast(kg[:, :Dh].astype(_BF16), _U32)
            g_v[rows, :] = kg[:, Dh:Dh + 1]

        def q_proj(r0, n, c0, nc):
            rows = slice(r0, r0 + n)
            cols = slice(c0, c0 + nc)
            q = jnp.dot(x_v[rows, :], wq_v[:, cols], preferred_element_type=_F32) * q_scale
            qtb = q.T.astype(_BF16)
            qtf = qtb.astype(_F32)
            lanes = slice(r0 % W, r0 % W + n)
            for h in range(c0 // Dh, (c0 + nc) // Dh):
                hr = slice(h * Dh - c0, (h + 1) * Dh - c0)
                qt_v[(r0 // W) * H + h, :, lanes] = qtb[hr, :]
                qf_v[(r0 // W) * H + h, :, lanes] = qtf[hr, :]

        x_copy(0).start()
        wq_copy(0).start()
        wq_copy(1).start()
        for j in range(3):
            w_copy(j).start()
        x_copy(0).wait()
        x_copy(1).start()
        wq_copy(0).wait()
        wq_copy(2).start()
        q_proj(0, 256, 0, QC)
        wq_copy(1).wait()
        for j in range(3):
            w_copy(j).wait()
        wq_copy(3).start()
        gw = gw_v[...].astype(_F32)
        first_row = lax.broadcasted_iota(jnp.int32, (GR, 128), 0) == 0
        for c in range(D // 128):
            tile = jnp.where(first_row, jnp.broadcast_to(gw[c:c + 1, :], (GR, 128)), 0.0)
            wkvt_v[Dh:V0, c * 128:(c + 1) * 128] = tile.astype(_BF16)
        q_proj(0, 256, QC, QC)
        x_copy(1).wait()
        x_copy(2).start()
        kv_proj(0, 512)
        q_proj(256, 256, 0, 2 * QC)
        wq_copy(2).wait()
        wq_copy(3).wait()
        x_copy(3).start()
        x_copy(4).start()
        q_proj(0, 512, 2 * QC, 2 * QC)
        x_copy(2).wait()
        for j in range(3, len(w_pairs)):
            w_copy(j).start()
        kv_proj(512, 512)
        q_proj(512, 512, 0, HD)
        x_copy(3).wait()
        x_copy(4).wait()
        kv_proj(1024, 512)
        kv_proj(1536, 512)
        for r0 in (1024, 1536):
            q_proj(r0, 512, 0, HD)
        kf = pltpu.bitcast(k_u[SM // 2:, :], _BF16).astype(_F32)
        for d in range(Dh):
            kb_v[d] = jnp.broadcast_to(kf[:, d:d + 1], (NV, 128))

        attn_group(0, None)
        kc = pltpu.bitcast(k_u[SM // 2:, :], _BF16)
        for g in range(G):
            s = jnp.dot(kc, qt_v[g], preferred_element_type=_F32)
            sv_v[g] = s
            s3 = s.reshape(NV // 8, 8, W)
            vm_v[g] = _tree(jnp.maximum, [s3[r] for r in range(NV // 8)])

        def ffn_part(q, chain):
            i = q // GF
            part = q % GF
            rows = pl.ds(pl.multiple_of(i * TM, TM), TM)
            items = []
            for j in range(NJ + 1):
                if j < NJ:
                    items.append(("gu", j, 2))
                if j >= 1:
                    items.append(("d", j - 1, 1))
            total = sum(it[2] for it in items)
            accum = 0
            hid = {}
            xt = x_v[rows, :]
            nf = len(pieces) - NA
            moved = False
            for kind, j, cost in items:
                cols = slice(j * _FS, (j + 1) * _FS)
                if kind == "gu":
                    gate = jnp.dot(xt, wg_v[part, :, cols], preferred_element_type=_F32)
                    up = jnp.dot(xt, wu_v[part, :, cols], preferred_element_type=_F32)
                    hid[j] = (jnp.maximum(gate, 0.0) * up).astype(_BF16)
                else:
                    dv = jnp.dot(hid.pop(j), wd_v[part, cols, :], preferred_element_type=_F32)
                    if j == 0:
                        bs_v[...] = jnp.where(part == 0, 0.0, bs_v[...]) + dv
                    elif j == NJ - 1:
                        tot = bs_v[...] + dv
                        bs_v[...] = tot
                        b_v[rows, :] = tot
                    else:
                        bs_v[...] += dv
                accum += cost
                chain[1](NA + (nf * accum + total - 1) // total)
                if not moved and pieces[min(chain[0]["done"], len(pieces) - 1)][0] > 0:
                    sv_v[0] = sv_v[G]
                    vm_v[0] = vm_v[G]
                    moved = True

        for j in range(3, 6):
            w_copy(j).wait()
        bs_v[...] = jnp.zeros_like(bs_v)

        def main_body(q, carry):
            for part in range(1, GF):
                @pl.when(q == part)
                def _():
                    for j in range(3 + 3 * part, 6 + 3 * part):
                        w_copy(j).wait()

            chain = make_chain(q + 1)
            attn_group((q + 1) * G, q * G, chain=chain)
            ffn_part(q, chain)
            return carry

        lax.fori_loop(0, NG - 1, main_body, 0)

        w_copy(len(w_pairs) - 1).wait()

        def transpose_o(r0, n):
            lanes = slice(r0 % W, r0 % W + n)
            ot = jnp.concatenate(
                [ot_v[(r0 // W) * H + h, :, lanes] for h in range(H)], axis=0)
            o_v[r0:r0 + n, :] = ot.T

        def oproj_piece(r0, n, c0, nc, prep):
            def f():
                rows = slice(r0, r0 + n)
                cols = slice(c0, c0 + nc)
                if prep:
                    transpose_o(r0, n)
                a = jnp.dot(o_v[rows, :], wo_v[:, cols], preferred_element_type=_F32)
                g = g_v[rows, :]
                out_v[rows, cols] = (g * a + (1.0 - g) * b_v[rows, cols]).astype(_BF16)
            return f

        def oproj_rows(lo, hi, prep):
            fs = []
            r0 = lo
            while r0 < hi:
                n = min(_OR, hi - r0)
                nc = _OC * _OR // n
                fs += [oproj_piece(r0, n, c0, nc, prep and c0 == 0) for c0 in range(0, D, nc)]
                r0 += n
            return fs

        def last_ffn_items():
            rows = slice(S - TM, S)
            hid = {}
            fs = []

            def gate(j):
                def f():
                    cols = slice(j * _FS, (j + 1) * _FS)
                    hid[j] = jnp.dot(x_v[rows, :], wg_v[GF - 1, :, cols],
                                     preferred_element_type=_F32)
                return f

            def up(j):
                def f():
                    cols = slice(j * _FS, (j + 1) * _FS)
                    u = jnp.dot(x_v[rows, :], wu_v[GF - 1, :, cols], preferred_element_type=_F32)
                    hid[j] = (jnp.maximum(hid[j], 0.0) * u).astype(_BF16)
                return f

            def down(j):
                def f():
                    cols = slice(j * _FS, (j + 1) * _FS)
                    dv = jnp.dot(hid.pop(j), wd_v[GF - 1, cols, :], preferred_element_type=_F32)
                    b_v[rows, :] += dv
                return f

            for j in range(NJ + 1):
                if j < NJ:
                    fs += [gate(j), up(j)]
                if j >= 1:
                    fs.append(down(j - 1))
            return fs

        fill = last_ffn_items() + oproj_rows(0, S - W, True)
        attn_group(None, NB - G, fill[:len(fill) - _HOLD])
        for r0 in range(S - W, S, _OR):
            transpose_o(r0, _OR)
        for f in fill[len(fill) - _HOLD:]:
            f()
        out_copy(0).start()
        for t in range(1, len(out_pieces)):
            r0, n = out_pieces[t]
            for f in oproj_rows(r0, r0 + n, False):
                f()
            out_copy(t).start()
        for t in range(len(out_pieces)):
            out_copy(t).wait()

    scratch = [
        pltpu.VMEM((S // 2, D), _U32),
        pltpu.VMEM((D // 2, HD), _U32),
        pltpu.VMEM(((V0 + Dh) // 2, D), _U32),
        pltpu.VMEM((HD // 2, D), _U32),
        pltpu.VMEM((GF, D // 2, FP), _U32),
        pltpu.VMEM((GF, D // 2, FP), _U32),
        pltpu.VMEM((GF, FP // 2, D), _U32),
        pltpu.VMEM((D // 128, 128), _BF16),
        pltpu.VMEM((NB, Dh // 2, W), _U32),
        pltpu.VMEM((S // 2, Dh), _U32),
        pltpu.VMEM((Dh // 2, S), _U32),
        pltpu.VMEM((NB, Dh // 2, W), _U32),
        pltpu.VMEM((S // 2, HD), _U32),
        pltpu.VMEM((S // 2, D), _U32),
        pltpu.VMEM((Dh, NV, 128), _F32),
        pltpu.VMEM((G + 1, NV, W), _F32),
        pltpu.VMEM((G + 1, 8, W), _F32),
        pltpu.VMEM((S, D), _F32),
        pltpu.VMEM((S, 1), _F32),
        pltpu.VMEM((NB, Dh, W), _F32),
        pltpu.VMEM((TM, D), _F32),
        pltpu.SemaphoreType.DMA((len(x_pieces),)),
        pltpu.SemaphoreType.DMA((4,)),
        pltpu.SemaphoreType.DMA((4 + 3 * GF,)),
        pltpu.SemaphoreType.DMA((len(out_pieces),)),
    ] + [pltpu.VMEM((SM, W), _F32)] * G + [pltpu.VMEM((8, W), _F32)] * G
    return kernel, scratch


@jax.jit
def pallas_gated_mix__grouped_kv_mqa__glu_gated_reglu__prompt_kernel(
    A_x: jax.Array,
    A_wq: jax.Array,
    A_wk: jax.Array,
    A_wv: jax.Array,
    A_wo: jax.Array,
    B_x: jax.Array,
    B_W_gate: jax.Array,
    B_W_up: jax.Array,
    B_W_down: jax.Array,
    gate_w: jax.Array,
):
    B, S, D = A_x.shape
    assert B == 1
    Dh = A_wk.shape[1]
    H = A_wq.shape[1] // Dh
    F = B_W_gate.shape[1]

    kernel, scratch = _make_kernel(S, D, H, Dh, F)
    any_spec = pl.BlockSpec(memory_space=pl.ANY)
    out = pl.pallas_call(
        kernel,
        in_specs=[any_spec] * 9,
        out_specs=any_spec,
        out_shape=jax.ShapeDtypeStruct((S, D), A_x.dtype),
        scratch_shapes=scratch,
        compiler_params=pltpu.CompilerParams(
            vmem_limit_bytes=120 * 1024 * 1024,
        ),
    )(A_x.reshape(S, D), A_wq, A_wk.T, A_wv.T, A_wo, B_W_gate, B_W_up, B_W_down,
      gate_w.reshape(D // 128, 128))
    return out.reshape(B, S, D)
```

```python
import math

import jax
import jax.numpy as jnp
from jax import lax
import jax.experimental.pallas as pl
import jax.experimental.pallas.tpu as pltpu

_F32 = jnp.float32
_BF16 = jnp.bfloat16
_U32 = jnp.uint32

_TM = 128
_W = 512
_KC = 128
_G = 4
_FS = 256
_OR = 256
_OC = 128
_NV = 224
_SA = (0, 0, 2, 1, 2, 2, 1, 1, 2, 1, 2, 1, 1, 0, 0, 0)
_PF = (2, 2, 3, 2, 3)
_DUE = 3
_C0 = 2
_LAST = 128
_HOLD = 4

_NT = (((1,), (1,)), ((), ()))


def _tree(op, parts):
    cur = list(parts)
    while len(cur) > 1:
        nxt = [op(cur[2 * j], cur[2 * j + 1]) for j in range(len(cur) // 2)]
        if len(cur) % 2:
            nxt.append(cur[-1])
        cur = nxt
    return cur[0]


def _zero_of(v):
    return jnp.minimum(jnp.maximum(v, 0.0), 0.0)


def _make_kernel(S, D, H, Dh, F):
    W, KC, G, TM, NV = _W, _KC, _G, _TM, _NV
    NB = H * (S // W)
    NC = S // KC
    R = KC // 8
    LT = W // 128
    HD = H * Dh
    SM = S - NV
    NF = S // TM
    NG = NB // G
    GF = NG // NF
    FP = F // GF
    NJ = FP // _FS
    assert NV % 16 == 0 and H % G == 0 and NG % NF == 0 and F % (_FS * GF) == 0
    assert len(_SA) == NC and S == 2048 and W == 512 and HD % 1024 == 0

    a_steps = [n for n in range(1, G * NC) if _SA[n % NC]]
    NA = len(a_steps)
    pieces = []
    for e in range(G):
        for j in range(LT):
            kk = 0
            while kk < NV:
                n = len(pieces)
                size = _SA[a_steps[n] % NC] if n < NA else _PF[(n - NA) % len(_PF)]
                kb = min(8 * size, NV - kk)
                pieces.append((e, kk, kb, j))
                kk += kb
    assert all(p[0] == 0 for p in pieces[:NA])

    n_big = NC - NV // 16
    assert n_big >= 0
    big = set((NC * t) // n_big for t in range(n_big))
    qk_rows = [KC if c in big else KC - 16 for c in range(NC)]
    qk_start = [sum(qk_rows[:c]) for c in range(NC)]
    q_scale = (Dh ** -0.5) * math.log2(math.e)
    x_pieces = [(0, 256), (256, 256), (512, 512), (1024, 512), (1536, 512)]
    QC = HD // 4
    out_pieces = [(0, S - W), (S - W, W - _LAST), (S - _LAST, _LAST)]
    GR = 16
    V0 = Dh + GR

    def kernel(x_hbm, wq_hbm, wkt_hbm, wvt_hbm, wo_hbm, wg_hbm, wu_hbm, wd_hbm, gw_hbm,
               out_hbm,
               x_u, wq_u, wkvt_u, wo_u, wg_u, wu_u, wd_u, gw_v,
               qt_u, k_u, vt_u, ot_u, o_u, out_u,
               kb_v, sv_v, vm_v, b_v, g_v, qf_v, bs_v,
               xsems, qsems, wsems, osems, *bufs):
        sbufs = bufs[:G]
        mbufs = bufs[G:]
        x_v, wq_v, wkvt_v, wo_v, wg_v, wu_v, wd_v, qt_v, vt_v, ot_v, o_v, out_v = [
            r.bitcast(_BF16) for r in
            (x_u, wq_u, wkvt_u, wo_u, wg_u, wu_u, wd_u, qt_u, vt_u, ot_u, o_u, out_u)]

        def x_copy(i):
            r0, n = x_pieces[i]
            return pltpu.make_async_copy(
                x_hbm.at[pl.ds(r0, n)], x_v.at[pl.ds(r0, n)], xsems.at[i])

        def wq_copy(j):
            return pltpu.make_async_copy(
                wq_hbm.at[:, pl.ds(j * QC, QC)], wq_v.at[:, pl.ds(j * QC, QC)], qsems.at[j])

        w_pairs = [(wkt_hbm, wkvt_v.at[pl.ds(0, Dh)]), (wvt_hbm, wkvt_v.at[pl.ds(V0, Dh)]),
                   (gw_hbm, gw_v)]
        for part in range(GF):
            fc = pl.ds(part * FP, FP)
            w_pairs += [(wg_hbm.at[:, fc], wg_v.at[part]), (wu_hbm.at[:, fc], wu_v.at[part]),
                        (wd_hbm.at[fc], wd_v.at[part])]
        w_pairs.append((wo_hbm, wo_v))

        def w_copy(j):
            return pltpu.make_async_copy(w_pairs[j][0], w_pairs[j][1], wsems.at[j])

        def out_copy(t):
            r0, n = out_pieces[t]
            return pltpu.make_async_copy(
                out_v.at[pl.ds(r0, n)], out_hbm.at[pl.ds(r0, n)], osems.at[t])

        def vpu_piece(b, slot, kk, kb, j, z):
            qblk = qf_v[b, :, j * 128:(j + 1) * 128]
            acc = z if kb == 8 else jnp.concatenate([z] * (kb // 8), axis=0)
            for d in range(Dh):
                t = kb_v[d, kk:kk + kb, :] * jnp.broadcast_to(qblk[d:d + 1, :], (kb, 128))
                acc = t + acc if d == 0 else acc + t
            sv_v[slot, kk:kk + kb, j * 128:(j + 1) * 128] = acc
            rows = [acc[r:r + 8, :] for r in range(0, kb, 8)]
            return _tree(jnp.maximum, rows), rows[0]

        def make_chain(grp):
            cs = dict(last=None, mv=None, done=0)

            def emit(upto):
                while cs["done"] < min(upto, len(pieces)):
                    e, kk, kb, j = pieces[cs["done"]]
                    slot = G if e == 0 else e
                    mxv, cs["last"] = vpu_piece(grp * G + e, slot, kk, kb, j, _zero_of(cs["last"]))
                    cs["mv"] = mxv if kk == 0 else jnp.maximum(cs["mv"], mxv)
                    if kk + kb == NV:
                        vm_v[slot, :, j * 128:(j + 1) * 128] = cs["mv"]
                    cs["done"] += 1
            return cs, emit

        def attn_group(b_next0, b_cur0, fillers=(), chain=None):
            do_qk = b_next0 is not None
            do_pv = b_cur0 is not None
            fillers = list(fillers)
            nfill = len(fillers)
            done = 0
            st = dict(mx=None, qt=None, m=None, acc=None, l=None)
            taps = []

            def load_scores(g, c):
                lo, hi = c * KC, (c + 1) * KC
                parts = []
                if lo < SM:
                    parts.append(sbufs[g][lo:min(hi, SM), :])
                if hi > SM:
                    parts.append(sv_v[g, max(lo, SM) - SM:hi - SM, :])
                sc = parts[0] if len(parts) == 1 else jnp.concatenate(parts, axis=0)
                if c == 0:
                    m = jnp.max(jnp.maximum(mbufs[g][...], vm_v[g]), axis=0, keepdims=True)
                    st["m"] = jnp.broadcast_to(m, (8, W))
                return sc.reshape(R, 8, W), st["m"]

            def qk(g, c):
                if c == 0:
                    st["qt"] = qt_v[b_next0 + g]
                    st["mx"] = None
                r0, n = qk_start[c], qk_rows[c]
                kc = pltpu.bitcast(k_u[r0 // 2:(r0 + n) // 2, :], _BF16)
                s = jnp.dot(kc, st["qt"], preferred_element_type=_F32)
                sbufs[g][r0:r0 + n, :] = s
                for r in range(0, n, 8):
                    sr = s[r:r + 8, :]
                    st["mx"] = sr if st["mx"] is None else jnp.maximum(st["mx"], sr)
                if c == NC - 1:
                    mbufs[g][...] = st["mx"]

            def pv(g, c, sc, m):
                lo, hi = c * KC, (c + 1) * KC
                if chain is not None:
                    ready = [v for (due, v) in taps if due <= g * NC + c]
                    taps[:] = [t for t in taps if t[0] > g * NC + c]
                    if c >= _C0:
                        link = st["l"]
                        if ready:
                            head = _tree(jnp.add, [link[:, :128]] + ready)
                            link = jnp.concatenate([head, link[:, 128:]], axis=1)
                        m = m + _zero_of(link)
                    elif ready:
                        head = m[:, :128] + _zero_of(_tree(jnp.add, ready))
                        m = jnp.concatenate([head, m[:, 128:]], axis=1)
                p = jnp.exp2(sc - m[None]).reshape(KC, W)
                t = _tree(jnp.add, [p[r:r + 8, :] for r in range(0, KC, 8)])
                st["l"] = t if c == 0 else st["l"] + t
                pb = p.astype(_BF16)
                d = jnp.dot(vt_v[:, lo:hi], pb, preferred_element_type=_F32)
                st["acc"] = d if c == 0 else st["acc"] + d
                if c == NC - 1:
                    lt = jnp.sum(st["l"], axis=0, keepdims=True)
                    ot_v[b_cur0 + g] = (st["acc"] * (1.0 / lt)).astype(_BF16)

            steps = [(g, c) for g in range(G) for c in range(NC)]
            pend = []
            for n, (g, c) in enumerate(steps):
                if do_pv:
                    pend.append((g, c) + load_scores(g, c))
                if do_qk:
                    qk(g, c)
                while done < nfill and done * len(steps) <= nfill * n:
                    fillers[done]()
                    done += 1
                if len(pend) > (1 if do_qk else 0):
                    pv(*pend.pop(0))
                if chain is not None and n in a_steps:
                    chain[0]["last"] = st["l"][:, :128]
                    chain[1](chain[0]["done"] + 1)
                    taps.append((n + _DUE, chain[0]["last"]))
            while pend:
                pv(*pend.pop(0))
            if chain is not None:
                chain[0]["last"] = st["l"][:, :128]
            while done < nfill:
                fillers[done]()
                done += 1

        def kv_proj(r0, n):
            rows = slice(r0, r0 + n)
            kvt = lax.dot_general(wkvt_v[...], x_v[rows, :], _NT, preferred_element_type=_F32)
            vt_v[:, rows] = kvt[V0:, :].astype(_BF16)
            kg = jnp.concatenate([kvt[:Dh, :], jax.nn.sigmoid(kvt[Dh:Dh + 8, :])], axis=0).T
            k_u[r0 // 2:(r0 + n) // 2, :] = pltpu.bitcast(kg[:, :Dh].astype(_BF16), _U32)
            g_v[rows, :] = kg[:, Dh:Dh + 1]

        def q_proj(r0, n, c0, nc):
            rows = slice(r0, r0 + n)
            cols = slice(c0, c0 + nc)
            q = jnp.dot(x_v[rows, :], wq_v[:, cols], preferred_element_type=_F32) * q_scale
            qtb = q.T.astype(_BF16)
            qtf = qtb.astype(_F32)
            lanes = slice(r0 % W, r0 % W + n)
            for h in range(c0 // Dh, (c0 + nc) // Dh):
                hr = slice(h * Dh - c0, (h + 1) * Dh - c0)
                qt_v[(r0 // W) * H + h, :, lanes] = qtb[hr, :]
                qf_v[(r0 // W) * H + h, :, lanes] = qtf[hr, :]

        x_copy(0).start()
        wq_copy(0).start()
        wq_copy(1).start()
        for j in range(3):
            w_copy(j).start()
        x_copy(0).wait()
        x_copy(1).start()
        wq_copy(0).wait()
        wq_copy(2).start()
        q_proj(0, 256, 0, QC)
        wq_copy(1).wait()
        for j in range(3):
            w_copy(j).wait()
        wq_copy(3).start()
        gw = gw_v[...].astype(_F32)
        first_row = lax.broadcasted_iota(jnp.int32, (GR, 128), 0) == 0
        for c in range(D // 128):
            tile = jnp.where(first_row, jnp.broadcast_to(gw[c:c + 1, :], (GR, 128)), 0.0)
            wkvt_v[Dh:V0, c * 128:(c + 1) * 128] = tile.astype(_BF16)
        q_proj(0, 256, QC, QC)
        x_copy(1).wait()
        x_copy(2).start()
        kv_proj(0, 512)
        q_proj(256, 256, 0, 2 * QC)
        wq_copy(2).wait()
        wq_copy(3).wait()
        x_copy(3).start()
        x_copy(4).start()
        q_proj(0, 512, 2 * QC, 2 * QC)
        x_copy(2).wait()
        for j in range(3, len(w_pairs)):
            w_copy(j).start()
        kv_proj(512, 512)
        q_proj(512, 512, 0, HD)
        x_copy(3).wait()
        x_copy(4).wait()
        kv_proj(1024, 512)
        kv_proj(1536, 512)
        for r0 in (1024, 1536):
            q_proj(r0, 512, 0, HD)
        kf = pltpu.bitcast(k_u[SM // 2:, :], _BF16).astype(_F32)
        for d in range(Dh):
            kb_v[d] = jnp.broadcast_to(kf[:, d:d + 1], (NV, 128))

        attn_group(0, None)
        kc = pltpu.bitcast(k_u[SM // 2:, :], _BF16)
        for g in range(G):
            s = jnp.dot(kc, qt_v[g], preferred_element_type=_F32)
            sv_v[g] = s
            s3 = s.reshape(NV // 8, 8, W)
            vm_v[g] = _tree(jnp.maximum, [s3[r] for r in range(NV // 8)])

        def ffn_part(q, chain):
            i = q // GF
            part = q % GF
            rows = pl.ds(pl.multiple_of(i * TM, TM), TM)
            items = []
            for j in range(NJ + 1):
                if j < NJ:
                    items.append(("gu", j, 2))
                if j >= 1:
                    items.append(("d", j - 1, 1))
            total = sum(it[2] for it in items)
            accum = 0
            hid = {}
            xt = x_v[rows, :]
            nf = len(pieces) - NA
            moved = False
            for kind, j, cost in items:
                cols = slice(j * _FS, (j + 1) * _FS)
                if kind == "gu":
                    gate = jnp.dot(xt, wg_v[part, :, cols], preferred_element_type=_F32)
                    up = jnp.dot(xt, wu_v[part, :, cols], preferred_element_type=_F32)
                    hid[j] = (jnp.maximum(gate, 0.0) * up).astype(_BF16)
                else:
                    dv = jnp.dot(hid.pop(j), wd_v[part, cols, :], preferred_element_type=_F32)
                    if j == 0:
                        bs_v[...] = jnp.where(part == 0, 0.0, bs_v[...]) + dv
                    elif j == NJ - 1:
                        tot = bs_v[...] + dv
                        bs_v[...] = tot
                        b_v[rows, :] = tot
                    else:
                        bs_v[...] += dv
                accum += cost
                chain[1](NA + (nf * accum + total - 1) // total)
                if not moved and pieces[min(chain[0]["done"], len(pieces) - 1)][0] > 0:
                    sv_v[0] = sv_v[G]
                    vm_v[0] = vm_v[G]
                    moved = True

        for j in range(3, 6):
            w_copy(j).wait()
        bs_v[...] = jnp.zeros_like(bs_v)

        def main_body(q, carry):
            for part in range(1, GF):
                @pl.when(q == part)
                def _():
                    for j in range(3 + 3 * part, 6 + 3 * part):
                        w_copy(j).wait()

            chain = make_chain(q + 1)
            attn_group((q + 1) * G, q * G, chain=chain)
            ffn_part(q, chain)
            return carry

        lax.fori_loop(0, NG - 1, main_body, 0)

        w_copy(len(w_pairs) - 1).wait()

        def transpose_o(r0, n):
            lanes = slice(r0 % W, r0 % W + n)
            ot = jnp.concatenate(
                [ot_v[(r0 // W) * H + h, :, lanes] for h in range(H)], axis=0)
            o_v[r0:r0 + n, :] = ot.T

        def oproj_piece(r0, n, c0, nc, prep):
            def f():
                rows = slice(r0, r0 + n)
                cols = slice(c0, c0 + nc)
                if prep:
                    transpose_o(r0, n)
                a = jnp.dot(o_v[rows, :], wo_v[:, cols], preferred_element_type=_F32)
                g = g_v[rows, :]
                out_v[rows, cols] = (g * a + (1.0 - g) * b_v[rows, cols]).astype(_BF16)
            return f

        def oproj_rows(lo, hi, prep):
            fs = []
            r0 = lo
            while r0 < hi:
                n = min(_OR, hi - r0)
                nc = _OC * _OR // n
                fs += [oproj_piece(r0, n, c0, nc, prep and c0 == 0) for c0 in range(0, D, nc)]
                r0 += n
            return fs

        def last_ffn_items():
            rows = slice(S - TM, S)
            hid = {}
            fs = []

            def gate(j):
                def f():
                    cols = slice(j * _FS, (j + 1) * _FS)
                    hid[j] = jnp.dot(x_v[rows, :], wg_v[GF - 1, :, cols],
                                     preferred_element_type=_F32)
                return f

            def up(j):
                def f():
                    cols = slice(j * _FS, (j + 1) * _FS)
                    u = jnp.dot(x_v[rows, :], wu_v[GF - 1, :, cols], preferred_element_type=_F32)
                    hid[j] = (jnp.maximum(hid[j], 0.0) * u).astype(_BF16)
                return f

            def down(j):
                def f():
                    cols = slice(j * _FS, (j + 1) * _FS)
                    dv = jnp.dot(hid.pop(j), wd_v[GF - 1, cols, :], preferred_element_type=_F32)
                    b_v[rows, :] += dv
                return f

            for j in range(NJ + 1):
                if j < NJ:
                    fs += [gate(j), up(j)]
                if j >= 1:
                    fs.append(down(j - 1))
            return fs

        fill = last_ffn_items() + oproj_rows(0, S - W, True)
        attn_group(None, NB - G, fill[:len(fill) - _HOLD])
        for r0 in range(S - W, S, _OR):
            transpose_o(r0, _OR)
        for f in fill[len(fill) - _HOLD:]:
            f()
        out_copy(0).start()
        for t in range(1, len(out_pieces)):
            r0, n = out_pieces[t]
            for f in oproj_rows(r0, r0 + n, False):
                f()
            out_copy(t).start()
        for t in range(len(out_pieces)):
            out_copy(t).wait()

    scratch = [
        pltpu.VMEM((S // 2, D), _U32),
        pltpu.VMEM((D // 2, HD), _U32),
        pltpu.VMEM(((V0 + Dh) // 2, D), _U32),
        pltpu.VMEM((HD // 2, D), _U32),
        pltpu.VMEM((GF, D // 2, FP), _U32),
        pltpu.VMEM((GF, D // 2, FP), _U32),
        pltpu.VMEM((GF, FP // 2, D), _U32),
        pltpu.VMEM((D // 128, 128), _BF16),
        pltpu.VMEM((NB, Dh // 2, W), _U32),
        pltpu.VMEM((S // 2, Dh), _U32),
        pltpu.VMEM((Dh // 2, S), _U32),
        pltpu.VMEM((NB, Dh // 2, W), _U32),
        pltpu.VMEM((S // 2, HD), _U32),
        pltpu.VMEM((S // 2, D), _U32),
        pltpu.VMEM((Dh, NV, 128), _F32),
        pltpu.VMEM((G + 1, NV, W), _F32),
        pltpu.VMEM((G + 1, 8, W), _F32),
        pltpu.VMEM((S, D), _F32),
        pltpu.VMEM((S, 1), _F32),
        pltpu.VMEM((NB, Dh, W), _F32),
        pltpu.VMEM((TM, D), _F32),
        pltpu.SemaphoreType.DMA((len(x_pieces),)),
        pltpu.SemaphoreType.DMA((4,)),
        pltpu.SemaphoreType.DMA((4 + 3 * GF,)),
        pltpu.SemaphoreType.DMA((len(out_pieces),)),
    ] + [pltpu.VMEM((SM, W), _F32)] * G + [pltpu.VMEM((8, W), _F32)] * G
    return kernel, scratch


@jax.jit
def pallas_gated_mix__grouped_kv_mqa__glu_gated_reglu__prompt_kernel(
    A_x: jax.Array,
    A_wq: jax.Array,
    A_wk: jax.Array,
    A_wv: jax.Array,
    A_wo: jax.Array,
    B_x: jax.Array,
    B_W_gate: jax.Array,
    B_W_up: jax.Array,
    B_W_down: jax.Array,
    gate_w: jax.Array,
):
    B, S, D = A_x.shape
    assert B == 1
    Dh = A_wk.shape[1]
    H = A_wq.shape[1] // Dh
    F = B_W_gate.shape[1]

    kernel, scratch = _make_kernel(S, D, H, Dh, F)
    any_spec = pl.BlockSpec(memory_space=pl.ANY)
    out = pl.pallas_call(
        kernel,
        in_specs=[any_spec] * 9,
        out_specs=any_spec,
        out_shape=jax.ShapeDtypeStruct((S, D), A_x.dtype),
        scratch_shapes=scratch,
        compiler_params=pltpu.CompilerParams(
            vmem_limit_bytes=120 * 1024 * 1024,
        ),
    )(A_x.reshape(S, D), A_wq, A_wk.T, A_wv.T, A_wo, B_W_gate, B_W_up, B_W_down,
      gate_w.reshape(D // 128, 128))
    return out.reshape(B, S, D)
```

```python
import math

import jax
import jax.numpy as jnp
from jax import lax
import jax.experimental.pallas as pl
import jax.experimental.pallas.tpu as pltpu

_F32 = jnp.float32
_BF16 = jnp.bfloat16
_U32 = jnp.uint32

_TM = 128
_W = 256
_KC = 128
_G = 8
_FS = 256
_OR = 256
_OC = 128
_NV = 256
_SA = (0, 0, 1, 1, 2, 1, 2, 1, 1, 1, 2, 1, 1, 0, 0, 0)
_PF = (2, 3)
_DUE = 3
_C0 = 1
_LATE = 512
_LAST = 128
_HOLD = 4

_NT = (((1,), (1,)), ((), ()))


def _tree(op, parts):
    cur = list(parts)
    while len(cur) > 1:
        nxt = [op(cur[2 * j], cur[2 * j + 1]) for j in range(len(cur) // 2)]
        if len(cur) % 2:
            nxt.append(cur[-1])
        cur = nxt
    return cur[0]


def _zero_of(v):
    return jnp.minimum(jnp.maximum(v, 0.0), 0.0)


def _make_kernel(S, D, H, Dh, F):
    W, KC, G, TM, NV = _W, _KC, _G, _TM, _NV
    NB = H * (S // W)
    NC = S // KC
    R = KC // 8
    LT = W // 128
    HD = H * Dh
    SM = S - NV
    NF = S // TM
    NG = NB // G
    GF = NG // NF
    FP = F // GF
    NJ = FP // _FS
    assert NV % 16 == 0 and H % G == 0 and NG % NF == 0 and F % (_FS * GF) == 0
    assert len(_SA) == NC and S == 2048 and W == 256 and _OR == W and HD % 1024 == 0

    a_steps = [n for n in range(1, G * NC) if _SA[n % NC]]
    NA = len(a_steps)
    pieces = []
    for e in range(G):
        for j in range(LT):
            kk = 0
            while kk < NV:
                n = len(pieces)
                size = _SA[a_steps[n] % NC] if n < NA else _PF[(n - NA) % len(_PF)]
                kb = min(8 * size, NV - kk)
                pieces.append((e, kk, kb, j))
                kk += kb
    assert all(p[0] == 0 or a_steps[t] >= (p[0] + 1) * NC for t, p in enumerate(pieces[:NA]))

    base, n_big = divmod(SM // 16, NC)
    big = set((NC * t) // n_big for t in range(n_big))
    qk_rows = [16 * (base + (c in big)) for c in range(NC)]
    assert all(sum(qk_rows[:c + 1]) <= KC * (c + 1) for c in range(NC))
    qk_start = [sum(qk_rows[:c]) for c in range(NC)]
    q_scale = (Dh ** -0.5) * math.log2(math.e)
    x_pieces = [(0, 256), (256, 256), (512, 512), (1024, 512), (1536, 512)]
    QC = HD // 4
    out_pieces = [(0, S - _LATE), (S - _LATE, _LATE - _LAST), (S - _LAST, _LAST)]
    GR = 16
    V0 = Dh + GR

    def kernel(x_hbm, wq_hbm, wkt_hbm, wvt_hbm, wo_hbm, wg_hbm, wu_hbm, wd_hbm, gw_hbm,
               out_hbm,
               x_u, wq_u, wkvt_u, wo_u, wg_u, wu_u, wd_u, gw_v,
               qt_u, k_u, vt_u, ot_u, o_u, out_u,
               kb_v, sv_v, vm_v, b_v, g_v, bs_v,
               xsems, qsems, wsems, osems, *bufs):
        sbufs = bufs[:G]
        mbufs = bufs[G:]
        x_v, wq_v, wkvt_v, wo_v, wg_v, wu_v, wd_v, qt_v, vt_v, ot_v, o_v, out_v = [
            r.bitcast(_BF16) for r in
            (x_u, wq_u, wkvt_u, wo_u, wg_u, wu_u, wd_u, qt_u, vt_u, ot_u, o_u, out_u)]

        def x_copy(i):
            r0, n = x_pieces[i]
            return pltpu.make_async_copy(
                x_hbm.at[pl.ds(r0, n)], x_v.at[pl.ds(r0, n)], xsems.at[i])

        def wq_copy(j):
            return pltpu.make_async_copy(
                wq_hbm.at[:, pl.ds(j * QC, QC)], wq_v.at[:, pl.ds(j * QC, QC)], qsems.at[j])

        w_pairs = [(wkt_hbm, wkvt_v.at[pl.ds(0, Dh)]), (wvt_hbm, wkvt_v.at[pl.ds(V0, Dh)]),
                   (gw_hbm, gw_v)]
        for part in range(GF):
            fc = pl.ds(part * FP, FP)
            w_pairs += [(wg_hbm.at[:, fc], wg_v.at[part]), (wu_hbm.at[:, fc], wu_v.at[part]),
                        (wd_hbm.at[fc], wd_v.at[part])]
        w_pairs.append((wo_hbm, wo_v))

        def w_copy(j):
            return pltpu.make_async_copy(w_pairs[j][0], w_pairs[j][1], wsems.at[j])

        def out_copy(t):
            r0, n = out_pieces[t]
            return pltpu.make_async_copy(
                out_v.at[pl.ds(r0, n)], out_hbm.at[pl.ds(r0, n)], osems.at[t])

        def vpu_piece(qblk, slot, kk, kb, j, z):
            acc = z if kb == 8 else jnp.concatenate([z] * (kb // 8), axis=0)
            for d in range(Dh):
                t = kb_v[d, kk:kk + kb, :] * jnp.broadcast_to(qblk[d:d + 1, :], (kb, 128))
                acc = t + acc if d == 0 else acc + t
            sv_v[slot, kk:kk + kb, j * 128:(j + 1) * 128] = acc
            rows = [acc[r:r + 8, :] for r in range(0, kb, 8)]
            return _tree(jnp.maximum, rows), rows[0]

        def make_chain(grp):
            cs = dict(last=None, mv=None, q=None, done=0)

            def emit(upto):
                while cs["done"] < min(upto, len(pieces)):
                    e, kk, kb, j = pieces[cs["done"]]
                    slot = G if e == 0 else e
                    if kk == 0:
                        cs["q"] = qt_v[grp * G + e][:, j * 128:(j + 1) * 128].astype(_F32)
                    mxv, cs["last"] = vpu_piece(cs["q"], slot, kk, kb, j, _zero_of(cs["last"]))
                    cs["mv"] = mxv if kk == 0 else jnp.maximum(cs["mv"], mxv)
                    if kk + kb == NV:
                        vm_v[slot, :, j * 128:(j + 1) * 128] = cs["mv"]
                    cs["done"] += 1
            return cs, emit

        def attn_group(q_next, b_cur0, fillers=(), chain=None):
            do_qk = q_next is not None
            do_pv = b_cur0 is not None
            fillers = list(fillers)
            nfill = len(fillers)
            done = 0
            st = dict(mx=None, qt=None, m=None, acc=None, l=None)
            taps = []

            def load_scores(g, c):
                lo, hi = c * KC, (c + 1) * KC
                parts = []
                if lo < SM:
                    parts.append(sbufs[g][lo:min(hi, SM), :])
                if hi > SM:
                    parts.append(sv_v[g, max(lo, SM) - SM:hi - SM, :])
                sc = parts[0] if len(parts) == 1 else jnp.concatenate(parts, axis=0)
                if c == 0:
                    m = jnp.max(jnp.maximum(mbufs[g][...], vm_v[g]), axis=0, keepdims=True)
                    st["m"] = jnp.broadcast_to(m, (8, W))
                return sc.reshape(R, 8, W), st["m"]

            def qk(g, c):
                if c == 0:
                    st["qt"] = q_next[g]
                    st["mx"] = None
                r0, n = qk_start[c], qk_rows[c]
                kc = pltpu.bitcast(k_u[r0 // 2:(r0 + n) // 2, :], _BF16)
                s = jnp.dot(kc, st["qt"], preferred_element_type=_F32)
                sbufs[g][r0:r0 + n, :] = s
                for r in range(0, n, 8):
                    sr = s[r:r + 8, :]
                    st["mx"] = sr if st["mx"] is None else jnp.maximum(st["mx"], sr)
                if c == NC - 1:
                    mbufs[g][...] = st["mx"]

            def pv(g, c, sc, m):
                lo, hi = c * KC, (c + 1) * KC
                if chain is not None:
                    ready = [v for (due, v) in taps if due <= g * NC + c]
                    taps[:] = [t for t in taps if t[0] > g * NC + c]
                    if c >= _C0:
                        link = st["l"]
                        if ready:
                            head = _tree(jnp.add, [link[:, :128]] + ready)
                            link = jnp.concatenate([head, link[:, 128:]], axis=1)
                        m = m + _zero_of(link)
                    elif ready:
                        head = m[:, :128] + _zero_of(_tree(jnp.add, ready))
                        m = jnp.concatenate([head, m[:, 128:]], axis=1)
                p = jnp.exp2(sc - m[None]).reshape(KC, W)
                t = _tree(jnp.add, [p[r:r + 8, :] for r in range(0, KC, 8)])
                st["l"] = t if c == 0 else st["l"] + t
                pb = p.astype(_BF16)
                d = jnp.dot(vt_v[:, lo:hi], pb, preferred_element_type=_F32)
                st["acc"] = d if c == 0 else st["acc"] + d
                if c == NC - 1:
                    lt = jnp.sum(st["l"], axis=0, keepdims=True)
                    ot_v[b_cur0 + g] = (st["acc"] * (1.0 / lt)).astype(_BF16)

            steps = [(g, c) for g in range(G) for c in range(NC)]
            pend = []
            for n, (g, c) in enumerate(steps):
                if do_pv:
                    pend.append((g, c) + load_scores(g, c))
                if do_qk:
                    qk(g, c)
                while done < nfill and done * len(steps) <= nfill * n:
                    fillers[done]()
                    done += 1
                if len(pend) > (1 if do_qk else 0):
                    pv(*pend.pop(0))
                if chain is not None and n in a_steps:
                    chain[0]["last"] = st["l"][:, :128]
                    chain[1](chain[0]["done"] + 1)
                    taps.append((n + _DUE, chain[0]["last"]))
            while pend:
                pv(*pend.pop(0))
            if chain is not None:
                chain[0]["last"] = st["l"][:, :128]
            while done < nfill:
                fillers[done]()
                done += 1

        def kv_proj(r0, n):
            rows = slice(r0, r0 + n)
            kvt = lax.dot_general(wkvt_v[...], x_v[rows, :], _NT, preferred_element_type=_F32)
            vt_v[:, rows] = kvt[V0:, :].astype(_BF16)
            kg = jnp.concatenate([kvt[:Dh, :], jax.nn.sigmoid(kvt[Dh:Dh + 8, :])], axis=0).T
            k_u[r0 // 2:(r0 + n) // 2, :] = pltpu.bitcast(kg[:, :Dh].astype(_BF16), _U32)
            g_v[rows, :] = kg[:, Dh:Dh + 1]

        def q_proj(r0, n, c0, nc):
            rows = slice(r0, r0 + n)
            cols = slice(c0, c0 + nc)
            q = jnp.dot(x_v[rows, :], wq_v[:, cols], preferred_element_type=_F32) * q_scale
            qtb = q.T.astype(_BF16)
            for o in range(0, n, W):
                for h in range(c0 // Dh, (c0 + nc) // Dh):
                    hr = slice(h * Dh - c0, (h + 1) * Dh - c0)
                    qt_v[((r0 + o) // W) * H + h] = qtb[hr, o:o + W]

        x_copy(0).start()
        wq_copy(0).start()
        wq_copy(1).start()
        for j in range(3):
            w_copy(j).start()
        x_copy(0).wait()
        x_copy(1).start()
        wq_copy(0).wait()
        wq_copy(2).start()
        q_proj(0, 256, 0, QC)
        wq_copy(1).wait()
        for j in range(3):
            w_copy(j).wait()
        wq_copy(3).start()
        gw = gw_v[...].astype(_F32)
        first_row = lax.broadcasted_iota(jnp.int32, (GR, 128), 0) == 0
        for c in range(D // 128):
            tile = jnp.where(first_row, jnp.broadcast_to(gw[c:c + 1, :], (GR, 128)), 0.0)
            wkvt_v[Dh:V0, c * 128:(c + 1) * 128] = tile.astype(_BF16)
        q_proj(0, 256, QC, QC)
        x_copy(1).wait()
        x_copy(2).start()
        kv_proj(0, 512)
        q_proj(256, 256, 0, 2 * QC)
        wq_copy(2).wait()
        wq_copy(3).wait()
        x_copy(3).start()
        x_copy(4).start()
        q_proj(0, 512, 2 * QC, 2 * QC)
        x_copy(2).wait()
        for j in range(3, len(w_pairs)):
            w_copy(j).start()
        kv_proj(512, 512)
        q_proj(512, 512, 0, HD)
        x_copy(3).wait()
        x_copy(4).wait()
        kv_proj(1024, 512)
        kv_proj(1536, 512)
        for r0 in (1024, 1536):
            q_proj(r0, 512, 0, HD)
        kf = pltpu.bitcast(k_u[SM // 2:, :], _BF16).astype(_F32)
        for d in range(Dh):
            kb_v[d] = jnp.broadcast_to(kf[:, d:d + 1], (NV, 128))

        attn_group(qt_v, None)
        kc = pltpu.bitcast(k_u[SM // 2:, :], _BF16)
        for g in range(G):
            s = jnp.dot(kc, qt_v[g], preferred_element_type=_F32)
            sv_v[g] = s
            s3 = s.reshape(NV // 8, 8, W)
            vm_v[g] = _tree(jnp.maximum, [s3[r] for r in range(NV // 8)])

        def ffn_part(q, chain):
            i = q // GF
            part = q % GF
            rows = pl.ds(pl.multiple_of(i * TM, TM), TM)
            items = []
            for j in range(NJ + 1):
                if j < NJ:
                    items.append(("gu", j, 2))
                if j >= 1:
                    items.append(("d", j - 1, 1))
            total = sum(it[2] for it in items)
            accum = 0
            hid = {}
            xt = x_v[rows, :]
            nf = len(pieces) - NA
            moved = False
            for kind, j, cost in items:
                cols = slice(j * _FS, (j + 1) * _FS)
                if kind == "gu":
                    gate = jnp.dot(xt, wg_v[part, :, cols], preferred_element_type=_F32)
                    up = jnp.dot(xt, wu_v[part, :, cols], preferred_element_type=_F32)
                    hid[j] = (jnp.maximum(gate, 0.0) * up).astype(_BF16)
                else:
                    dv = jnp.dot(hid.pop(j), wd_v[part, cols, :], preferred_element_type=_F32)
                    if j == 0:
                        bs_v[...] = jnp.where(part == 0, 0.0, bs_v[...]) + dv
                    elif j == NJ - 1:
                        tot = bs_v[...] + dv
                        bs_v[...] = tot
                        b_v[rows, :] = tot
                    else:
                        bs_v[...] += dv
                accum += cost
                chain[1](NA + (nf * accum + total - 1) // total)
                if not moved and pieces[min(chain[0]["done"], len(pieces) - 1)][0] > 0:
                    sv_v[0] = sv_v[G]
                    vm_v[0] = vm_v[G]
                    moved = True

        for j in range(3, 6):
            w_copy(j).wait()
        bs_v[...] = jnp.zeros_like(bs_v)

        def main_body(q, carry):
            for part in range(1, GF):
                @pl.when(q == part)
                def _():
                    for j in range(3 + 3 * part, 6 + 3 * part):
                        w_copy(j).wait()

            chain = make_chain(q + 1)
            attn_group(qt_v.at[pl.ds((q + 1) * G, G)], q * G, chain=chain)
            ffn_part(q, chain)
            return carry

        lax.fori_loop(0, NG - 1, main_body, 0)

        w_copy(len(w_pairs) - 1).wait()

        def transpose_o(r0, n):
            lanes = slice(r0 % W, r0 % W + n)
            ot = jnp.concatenate(
                [ot_v[(r0 // W) * H + h, :, lanes] for h in range(H)], axis=0)
            o_v[r0:r0 + n, :] = ot.T

        def oproj_piece(r0, n, c0, nc, prep):
            def f():
                rows = slice(r0, r0 + n)
                cols = slice(c0, c0 + nc)
                if prep:
                    transpose_o(r0, n)
                a = jnp.dot(o_v[rows, :], wo_v[:, cols], preferred_element_type=_F32)
                g = g_v[rows, :]
                out_v[rows, cols] = (g * a + (1.0 - g) * b_v[rows, cols]).astype(_BF16)
            return f

        def oproj_rows(lo, hi, prep):
            fs = []
            r0 = lo
            while r0 < hi:
                n = min(_OR, hi - r0)
                nc = _OC * _OR // n
                fs += [oproj_piece(r0, n, c0, nc, prep and c0 == 0) for c0 in range(0, D, nc)]
                r0 += n
            return fs

        def last_ffn_items():
            rows = slice(S - TM, S)
            hid = {}
            fs = []

            def gate(j):
                def f():
                    cols = slice(j * _FS, (j + 1) * _FS)
                    hid[j] = jnp.dot(x_v[rows, :], wg_v[GF - 1, :, cols],
                                     preferred_element_type=_F32)
                return f

            def up(j):
                def f():
                    cols = slice(j * _FS, (j + 1) * _FS)
                    u = jnp.dot(x_v[rows, :], wu_v[GF - 1, :, cols], preferred_element_type=_F32)
                    hid[j] = (jnp.maximum(hid[j], 0.0) * u).astype(_BF16)
                return f

            def down(j):
                def f():
                    cols = slice(j * _FS, (j + 1) * _FS)
                    dv = jnp.dot(hid.pop(j), wd_v[GF - 1, cols, :], preferred_element_type=_F32)
                    b_v[rows, :] += dv
                return f

            for j in range(NJ + 1):
                if j < NJ:
                    fs += [gate(j), up(j)]
                if j >= 1:
                    fs.append(down(j - 1))
            return fs

        fill = last_ffn_items() + oproj_rows(0, S - _LATE, True)
        attn_group(None, NB - G, fill[:len(fill) - _HOLD])
        for r0 in range(S - _LATE, S, _OR):
            transpose_o(r0, _OR)
        for f in fill[len(fill) - _HOLD:]:
            f()
        out_copy(0).start()
        for t in range(1, len(out_pieces)):
            r0, n = out_pieces[t]
            for f in oproj_rows(r0, r0 + n, False):
                f()
            out_copy(t).start()
        for t in range(len(out_pieces)):
            out_copy(t).wait()

    scratch = [
        pltpu.VMEM((S // 2, D), _U32),
        pltpu.VMEM((D // 2, HD), _U32),
        pltpu.VMEM(((V0 + Dh) // 2, D), _U32),
        pltpu.VMEM((HD // 2, D), _U32),
        pltpu.VMEM((GF, D // 2, FP), _U32),
        pltpu.VMEM((GF, D // 2, FP), _U32),
        pltpu.VMEM((GF, FP // 2, D), _U32),
        pltpu.VMEM((D // 128, 128), _BF16),
        pltpu.VMEM((NB, Dh // 2, W), _U32),
        pltpu.VMEM((S // 2, Dh), _U32),
        pltpu.VMEM((Dh // 2, S), _U32),
        pltpu.VMEM((NB, Dh // 2, W), _U32),
        pltpu.VMEM((S // 2, HD), _U32),
        pltpu.VMEM((S // 2, D), _U32),
        pltpu.VMEM((Dh, NV, 128), _F32),
        pltpu.VMEM((G + 1, NV, W), _F32),
        pltpu.VMEM((G + 1, 8, W), _F32),
        pltpu.VMEM((S, D), _F32),
        pltpu.VMEM((S, 1), _F32),
        pltpu.VMEM((TM, D), _F32),
        pltpu.SemaphoreType.DMA((len(x_pieces),)),
        pltpu.SemaphoreType.DMA((4,)),
        pltpu.SemaphoreType.DMA((4 + 3 * GF,)),
        pltpu.SemaphoreType.DMA((len(out_pieces),)),
    ] + [pltpu.VMEM((SM, W), _F32)] * G + [pltpu.VMEM((8, W), _F32)] * G
    return kernel, scratch


@jax.jit
def pallas_gated_mix__grouped_kv_mqa__glu_gated_reglu__prompt_kernel(
    A_x: jax.Array,
    A_wq: jax.Array,
    A_wk: jax.Array,
    A_wv: jax.Array,
    A_wo: jax.Array,
    B_x: jax.Array,
    B_W_gate: jax.Array,
    B_W_up: jax.Array,
    B_W_down: jax.Array,
    gate_w: jax.Array,
):
    B, S, D = A_x.shape
    assert B == 1
    Dh = A_wk.shape[1]
    H = A_wq.shape[1] // Dh
    F = B_W_gate.shape[1]

    kernel, scratch = _make_kernel(S, D, H, Dh, F)
    any_spec = pl.BlockSpec(memory_space=pl.ANY)
    out = pl.pallas_call(
        kernel,
        in_specs=[any_spec] * 9,
        out_specs=any_spec,
        out_shape=jax.ShapeDtypeStruct((S, D), A_x.dtype),
        scratch_shapes=scratch,
        compiler_params=pltpu.CompilerParams(
            vmem_limit_bytes=120 * 1024 * 1024,
        ),
    )(A_x.reshape(S, D), A_wq, A_wk.T, A_wv.T, A_wo, B_W_gate, B_W_up, B_W_down,
      gate_w.reshape(D // 128, 128))
    return out.reshape(B, S, D)
```

```python
import math

import jax
import jax.numpy as jnp
from jax import lax
import jax.experimental.pallas as pl
import jax.experimental.pallas.tpu as pltpu

_F32 = jnp.float32
_BF16 = jnp.bfloat16
_U32 = jnp.uint32

_TM = 128
_W = 256
_KC = 128
_G = 8
_FS = 256
_OR = 256
_OC = 128
_NV = 256
_SA = (0, 0, 1, 1, 2, 1, 2, 1, 1, 1, 2, 1, 1, 0, 0, 0)
_PF = (2, 3)
_DUE = 3
_C0 = 1
_LATE = 512
_LAST = 128
_PARK = 128
_HOLD = 4

_NT = (((1,), (1,)), ((), ()))


def _tree(op, parts):
    cur = list(parts)
    while len(cur) > 1:
        nxt = [op(cur[2 * j], cur[2 * j + 1]) for j in range(len(cur) // 2)]
        if len(cur) % 2:
            nxt.append(cur[-1])
        cur = nxt
    return cur[0]


def _zero_of(v):
    return jnp.minimum(jnp.maximum(v, 0.0), 0.0)


def _make_kernel(S, D, H, Dh, F):
    W, KC, G, TM, NV = _W, _KC, _G, _TM, _NV
    NB = H * (S // W)
    NC = S // KC
    R = KC // 8
    LT = W // 128
    HD = H * Dh
    SM = S - NV
    NF = S // TM
    NG = NB // G
    GF = NG // NF
    FP = F // GF
    NJ = FP // _FS
    assert NV % 16 == 0 and H % G == 0 and NG % NF == 0 and F % (_FS * GF) == 0
    assert len(_SA) == NC and S == 2048 and W == 256 and _OR == W and HD % 1024 == 0

    a_steps = [n for n in range(1, G * NC) if _SA[n % NC]]
    NA = len(a_steps)
    pieces = []
    for e in range(G):
        for j in range(LT):
            kk = 0
            while kk < NV:
                n = len(pieces)
                size = _SA[a_steps[n] % NC] if n < NA else _PF[(n - NA) % len(_PF)]
                kb = min(8 * size, NV - kk)
                pieces.append((e, kk, kb, j))
                kk += kb
    assert all(p[0] == 0 or a_steps[t] >= (p[0] + 1) * NC for t, p in enumerate(pieces[:NA]))

    base, n_big = divmod(SM // 16, NC)
    big = set((NC * t) // n_big for t in range(n_big))
    qk_rows = [16 * (base + (c in big)) for c in range(NC)]
    assert all(sum(qk_rows[:c + 1]) <= KC * (c + 1) for c in range(NC))
    qk_start = [sum(qk_rows[:c]) for c in range(NC)]
    q_scale = (Dh ** -0.5) * math.log2(math.e)
    x_pieces = [(0, 256), (256, 256), (512, 512), (1024, 512), (1536, 512)]
    QC = HD // 4
    out_pieces = [(0, S - _LATE), (S - _LATE, _LATE - _LAST), (S - _LAST, _LAST)]
    GR = 16
    V0 = Dh + GR

    def kernel(x_hbm, wq_hbm, wkt_hbm, wvt_hbm, wo_hbm, wg_hbm, wu_hbm, wd_hbm, gw_hbm,
               out_hbm,
               x_u, wq_u, wkvt_u, wo_u, wg_u, wu_u, wd_u, gw_v,
               qt_u, k_u, vt_u, ot_u, o_u, out_u,
               kb_v, sv_v, vm_v, b_v, g_v, bs_v, park_v,
               xsems, qsems, wsems, osems, *bufs):
        sbufs = bufs[:G]
        mbufs = bufs[G:]
        x_v, wq_v, wkvt_v, wo_v, wg_v, wu_v, wd_v, qt_v, vt_v, ot_v, o_v, out_v = [
            r.bitcast(_BF16) for r in
            (x_u, wq_u, wkvt_u, wo_u, wg_u, wu_u, wd_u, qt_u, vt_u, ot_u, o_u, out_u)]

        def x_copy(i):
            r0, n = x_pieces[i]
            return pltpu.make_async_copy(
                x_hbm.at[pl.ds(r0, n)], x_v.at[pl.ds(r0, n)], xsems.at[i])

        def wq_copy(j):
            return pltpu.make_async_copy(
                wq_hbm.at[:, pl.ds(j * QC, QC)], wq_v.at[:, pl.ds(j * QC, QC)], qsems.at[j])

        w_pairs = [(wkt_hbm, wkvt_v.at[pl.ds(0, Dh)]), (wvt_hbm, wkvt_v.at[pl.ds(V0, Dh)]),
                   (gw_hbm, gw_v)]
        for part in range(GF):
            fc = pl.ds(part * FP, FP)
            w_pairs += [(wg_hbm.at[:, fc], wg_v.at[part]), (wu_hbm.at[:, fc], wu_v.at[part]),
                        (wd_hbm.at[fc], wd_v.at[part])]
        w_pairs.append((wo_hbm, wo_v))

        def w_copy(j):
            return pltpu.make_async_copy(w_pairs[j][0], w_pairs[j][1], wsems.at[j])

        def out_copy(t):
            r0, n = out_pieces[t]
            return pltpu.make_async_copy(
                out_v.at[pl.ds(r0, n)], out_hbm.at[pl.ds(r0, n)], osems.at[t])

        def vpu_piece(qblk, slot, kk, kb, j, z):
            acc = z if kb == 8 else jnp.concatenate([z] * (kb // 8), axis=0)
            for d in range(Dh):
                t = kb_v[d, kk:kk + kb, :] * jnp.broadcast_to(qblk[d:d + 1, :], (kb, 128))
                acc = t + acc if d == 0 else acc + t
            sv_v[slot, kk:kk + kb, j * 128:(j + 1) * 128] = acc
            rows = [acc[r:r + 8, :] for r in range(0, kb, 8)]
            return _tree(jnp.maximum, rows), rows[0]

        def make_chain(grp):
            cs = dict(last=None, mv=None, q=None, done=0)

            def emit(upto):
                while cs["done"] < min(upto, len(pieces)):
                    e, kk, kb, j = pieces[cs["done"]]
                    slot = G if e == 0 else e
                    if kk == 0:
                        cs["q"] = qt_v[grp * G + e][:, j * 128:(j + 1) * 128].astype(_F32)
                    mxv, cs["last"] = vpu_piece(cs["q"], slot, kk, kb, j, _zero_of(cs["last"]))
                    cs["mv"] = mxv if kk == 0 else jnp.maximum(cs["mv"], mxv)
                    if kk + kb == NV:
                        vm_v[slot, :, j * 128:(j + 1) * 128] = cs["mv"]
                    cs["done"] += 1
            return cs, emit

        def attn_group(q_next, b_cur0, fillers=(), chain=None):
            do_qk = q_next is not None
            do_pv = b_cur0 is not None
            fillers = list(fillers)
            nfill = len(fillers)
            done = 0
            st = dict(mx=None, qt=None, m=None, acc=None, l=None)
            taps = []

            def load_scores(g, c):
                lo, hi = c * KC, (c + 1) * KC
                parts = []
                if lo < SM:
                    parts.append(sbufs[g][lo:min(hi, SM), :])
                if hi > SM:
                    parts.append(sv_v[g, max(lo, SM) - SM:hi - SM, :])
                sc = parts[0] if len(parts) == 1 else jnp.concatenate(parts, axis=0)
                if c == 0:
                    m = jnp.max(jnp.maximum(mbufs[g][...], vm_v[g]), axis=0, keepdims=True)
                    st["m"] = jnp.broadcast_to(m, (8, W))
                return sc.reshape(R, 8, W), st["m"]

            def qk(g, c):
                if c == 0:
                    st["qt"] = q_next[g]
                    st["mx"] = None
                r0, n = qk_start[c], qk_rows[c]
                kc = pltpu.bitcast(k_u[r0 // 2:(r0 + n) // 2, :], _BF16)
                s = jnp.dot(kc, st["qt"], preferred_element_type=_F32)
                sbufs[g][r0:r0 + n, :] = s
                for r in range(0, n, 8):
                    sr = s[r:r + 8, :]
                    st["mx"] = sr if st["mx"] is None else jnp.maximum(st["mx"], sr)
                if c == NC - 1:
                    mbufs[g][...] = st["mx"]

            def pv(g, c, sc, m):
                lo, hi = c * KC, (c + 1) * KC
                if chain is not None:
                    ready = [v for (due, v) in taps if due <= g * NC + c]
                    taps[:] = [t for t in taps if t[0] > g * NC + c]
                    if c >= _C0:
                        link = st["l"]
                        if ready:
                            head = _tree(jnp.add, [link[:, :128]] + ready)
                            link = jnp.concatenate([head, link[:, 128:]], axis=1)
                        m = m + _zero_of(link)
                    elif ready:
                        head = m[:, :128] + _zero_of(_tree(jnp.add, ready))
                        m = jnp.concatenate([head, m[:, 128:]], axis=1)
                p = jnp.exp2(sc - m[None]).reshape(KC, W)
                t = _tree(jnp.add, [p[r:r + 8, :] for r in range(0, KC, 8)])
                st["l"] = t if c == 0 else st["l"] + t
                pb = p.astype(_BF16)
                d = jnp.dot(vt_v[:, lo:hi], pb, preferred_element_type=_F32)
                st["acc"] = d if c == 0 else st["acc"] + d
                if c == NC - 1:
                    lt = jnp.sum(st["l"], axis=0, keepdims=True)
                    ot_v[b_cur0 + g] = (st["acc"] * (1.0 / lt)).astype(_BF16)

            steps = [(g, c) for g in range(G) for c in range(NC)]
            pend = []
            for n, (g, c) in enumerate(steps):
                if do_pv:
                    pend.append((g, c) + load_scores(g, c))
                if do_qk:
                    qk(g, c)
                while done < nfill and done * len(steps) <= nfill * n:
                    fillers[done]()
                    done += 1
                if len(pend) > (1 if do_qk else 0):
                    pv(*pend.pop(0))
                if chain is not None and n in a_steps:
                    chain[0]["last"] = st["l"][:, :128]
                    chain[1](chain[0]["done"] + 1)
                    taps.append((n + _DUE, chain[0]["last"]))
            while pend:
                pv(*pend.pop(0))
            if chain is not None:
                chain[0]["last"] = st["l"][:, :128]
            while done < nfill:
                fillers[done]()
                done += 1

        def kv_proj(r0, n):
            rows = slice(r0, r0 + n)
            kvt = lax.dot_general(wkvt_v[...], x_v[rows, :], _NT, preferred_element_type=_F32)
            vt_v[:, rows] = kvt[V0:, :].astype(_BF16)
            kg = jnp.concatenate([kvt[:Dh, :], jax.nn.sigmoid(kvt[Dh:Dh + 8, :])], axis=0).T
            k_u[r0 // 2:(r0 + n) // 2, :] = pltpu.bitcast(kg[:, :Dh].astype(_BF16), _U32)
            g_v[rows, :] = kg[:, Dh:Dh + 1]

        def q_store(q, r0, n, c0, nc):
            qtb = q.T.astype(_BF16)
            for o in range(0, n, W):
                for h in range(c0 // Dh, (c0 + nc) // Dh):
                    hr = slice(h * Dh - c0, (h + 1) * Dh - c0)
                    qt_v[((r0 + o) // W) * H + h] = qtb[hr, o:o + W]

        def q_mm(r0, n, c0, nc):
            return jnp.dot(x_v[r0:r0 + n, :], wq_v[:, c0:c0 + nc],
                           preferred_element_type=_F32) * q_scale

        def q_proj(r0, n, c0, nc):
            q_store(q_mm(r0, n, c0, nc), r0, n, c0, nc)

        def q_proj_parked(r0, n, c0, nc):
            if nc > _PARK:
                q_proj(r0, n, c0, nc - _PARK)
            c1 = c0 + nc - _PARK
            park_v[0:n, :] = q_mm(r0, n, c1, _PARK)
            return lambda: q_store(park_v[0:n, :], r0, n, c1, _PARK)

        x_copy(0).start()
        for j in range(3):
            w_copy(j).start()
        wq_copy(0).start()
        wq_copy(1).start()
        bs_v[...] = jnp.zeros_like(bs_v)
        x_copy(0).wait()
        for j in range(3):
            w_copy(j).wait()
        x_copy(1).start()
        gw = gw_v[...].astype(_F32)
        first_row = lax.broadcasted_iota(jnp.int32, (GR, 128), 0) == 0
        for c in range(D // 128):
            tile = jnp.where(first_row, jnp.broadcast_to(gw[c:c + 1, :], (GR, 128)), 0.0)
            wkvt_v[Dh:V0, c * 128:(c + 1) * 128] = tile.astype(_BF16)
        kv_proj(0, 256)
        wq_copy(0).wait()
        wq_copy(2).start()
        finish = q_proj_parked(0, 256, 0, QC)
        wq_copy(1).wait()
        wq_copy(3).start()
        finish()
        finish = q_proj_parked(0, 256, QC, QC)
        x_copy(1).wait()
        x_copy(2).start()
        finish()
        kv_proj(256, 256)
        finish = q_proj_parked(256, 256, 0, 2 * QC)
        wq_copy(2).wait()
        wq_copy(3).wait()
        x_copy(3).start()
        x_copy(4).start()
        finish()
        finish = q_proj_parked(0, 512, 2 * QC, 2 * QC)
        x_copy(2).wait()
        for j in range(3, len(w_pairs)):
            w_copy(j).start()
        finish()
        kv_proj(512, 512)
        finish = q_proj_parked(512, 512, 0, HD)
        x_copy(3).wait()
        x_copy(4).wait()
        finish()
        kv_proj(1024, 512)
        kv_proj(1536, 512)
        for r0 in (1024, 1536):
            q_proj(r0, 512, 0, HD)
        kf = pltpu.bitcast(k_u[SM // 2:, :], _BF16).astype(_F32)
        for d in range(Dh):
            kb_v[d] = jnp.broadcast_to(kf[:, d:d + 1], (NV, 128))

        attn_group(qt_v, None)
        kc = pltpu.bitcast(k_u[SM // 2:, :], _BF16)
        for g in range(G):
            s = jnp.dot(kc, qt_v[g], preferred_element_type=_F32)
            sv_v[g] = s
            s3 = s.reshape(NV // 8, 8, W)
            vm_v[g] = _tree(jnp.maximum, [s3[r] for r in range(NV // 8)])

        def ffn_part(q, chain):
            i = q // GF
            part = q % GF
            rows = pl.ds(pl.multiple_of(i * TM, TM), TM)
            items = []
            for j in range(NJ + 1):
                if j < NJ:
                    items.append(("gu", j, 2))
                if j >= 1:
                    items.append(("d", j - 1, 1))
            total = sum(it[2] for it in items)
            accum = 0
            hid = {}
            xt = x_v[rows, :]
            nf = len(pieces) - NA
            moved = False
            for kind, j, cost in items:
                cols = slice(j * _FS, (j + 1) * _FS)
                if kind == "gu":
                    gate = jnp.dot(xt, wg_v[part, :, cols], preferred_element_type=_F32)
                    up = jnp.dot(xt, wu_v[part, :, cols], preferred_element_type=_F32)
                    hid[j] = (jnp.maximum(gate, 0.0) * up).astype(_BF16)
                else:
                    dv = jnp.dot(hid.pop(j), wd_v[part, cols, :], preferred_element_type=_F32)
                    if j == 0:
                        bs_v[...] = jnp.where(part == 0, 0.0, bs_v[...]) + dv
                    elif j == NJ - 1:
                        tot = bs_v[...] + dv
                        bs_v[...] = tot
                        b_v[rows, :] = tot
                    else:
                        bs_v[...] += dv
                accum += cost
                chain[1](NA + (nf * accum + total - 1) // total)
                if not moved and pieces[min(chain[0]["done"], len(pieces) - 1)][0] > 0:
                    sv_v[0] = sv_v[G]
                    vm_v[0] = vm_v[G]
                    moved = True

        for j in range(3, 6):
            w_copy(j).wait()

        def main_body(q, carry):
            for part in range(1, GF):
                @pl.when(q == part)
                def _():
                    for j in range(3 + 3 * part, 6 + 3 * part):
                        w_copy(j).wait()

            chain = make_chain(q + 1)
            attn_group(qt_v.at[pl.ds((q + 1) * G, G)], q * G, chain=chain)
            ffn_part(q, chain)
            return carry

        lax.fori_loop(0, NG - 1, main_body, 0)

        w_copy(len(w_pairs) - 1).wait()

        def transpose_o(r0, n):
            lanes = slice(r0 % W, r0 % W + n)
            ot = jnp.concatenate(
                [ot_v[(r0 // W) * H + h, :, lanes] for h in range(H)], axis=0)
            o_v[r0:r0 + n, :] = ot.T

        def oproj_piece(r0, n, c0, nc, prep):
            def f():
                rows = slice(r0, r0 + n)
                cols = slice(c0, c0 + nc)
                if prep:
                    transpose_o(r0, n)
                a = jnp.dot(o_v[rows, :], wo_v[:, cols], preferred_element_type=_F32)
                g = g_v[rows, :]
                out_v[rows, cols] = (g * a + (1.0 - g) * b_v[rows, cols]).astype(_BF16)
            return f

        def oproj_rows(lo, hi, prep):
            fs = []
            r0 = lo
            while r0 < hi:
                n = min(_OR, hi - r0)
                nc = _OC * _OR // n
                fs += [oproj_piece(r0, n, c0, nc, prep and c0 == 0) for c0 in range(0, D, nc)]
                r0 += n
            return fs

        def last_ffn_items():
            rows = slice(S - TM, S)
            hid = {}
            fs = []

            def gate(j):
                def f():
                    cols = slice(j * _FS, (j + 1) * _FS)
                    hid[j] = jnp.dot(x_v[rows, :], wg_v[GF - 1, :, cols],
                                     preferred_element_type=_F32)
                return f

            def up(j):
                def f():
                    cols = slice(j * _FS, (j + 1) * _FS)
                    u = jnp.dot(x_v[rows, :], wu_v[GF - 1, :, cols], preferred_element_type=_F32)
                    hid[j] = (jnp.maximum(hid[j], 0.0) * u).astype(_BF16)
                return f

            def down(j):
                def f():
                    cols = slice(j * _FS, (j + 1) * _FS)
                    dv = jnp.dot(hid.pop(j), wd_v[GF - 1, cols, :], preferred_element_type=_F32)
                    b_v[rows, :] += dv
                return f

            for j in range(NJ + 1):
                if j < NJ:
                    fs += [gate(j), up(j)]
                if j >= 1:
                    fs.append(down(j - 1))
            return fs

        fill = last_ffn_items() + oproj_rows(0, S - _LATE, True)
        attn_group(None, NB - G, fill[:len(fill) - _HOLD])
        for r0 in range(S - _LATE, S, _OR):
            transpose_o(r0, _OR)
        for f in fill[len(fill) - _HOLD:]:
            f()
        out_copy(0).start()
        for t in range(1, len(out_pieces)):
            r0, n = out_pieces[t]
            for f in oproj_rows(r0, r0 + n, False):
                f()
            out_copy(t).start()
        for t in range(len(out_pieces)):
            out_copy(t).wait()

    scratch = [
        pltpu.VMEM((S // 2, D), _U32),
        pltpu.VMEM((D // 2, HD), _U32),
        pltpu.VMEM(((V0 + Dh) // 2, D), _U32),
        pltpu.VMEM((HD // 2, D), _U32),
        pltpu.VMEM((GF, D // 2, FP), _U32),
        pltpu.VMEM((GF, D // 2, FP), _U32),
        pltpu.VMEM((GF, FP // 2, D), _U32),
        pltpu.VMEM((D // 128, 128), _BF16),
        pltpu.VMEM((NB, Dh // 2, W), _U32),
        pltpu.VMEM((S // 2, Dh), _U32),
        pltpu.VMEM((Dh // 2, S), _U32),
        pltpu.VMEM((NB, Dh // 2, W), _U32),
        pltpu.VMEM((S // 2, HD), _U32),
        pltpu.VMEM((S // 2, D), _U32),
        pltpu.VMEM((Dh, NV, 128), _F32),
        pltpu.VMEM((G + 1, NV, W), _F32),
        pltpu.VMEM((G + 1, 8, W), _F32),
        pltpu.VMEM((S, D), _F32),
        pltpu.VMEM((S, 1), _F32),
        pltpu.VMEM((TM, D), _F32),
        pltpu.VMEM((512, _PARK), _F32),
        pltpu.SemaphoreType.DMA((len(x_pieces),)),
        pltpu.SemaphoreType.DMA((4,)),
        pltpu.SemaphoreType.DMA((4 + 3 * GF,)),
        pltpu.SemaphoreType.DMA((len(out_pieces),)),
    ] + [pltpu.VMEM((SM, W), _F32)] * G + [pltpu.VMEM((8, W), _F32)] * G
    return kernel, scratch


@jax.jit
def pallas_gated_mix__grouped_kv_mqa__glu_gated_reglu__prompt_kernel(
    A_x: jax.Array,
    A_wq: jax.Array,
    A_wk: jax.Array,
    A_wv: jax.Array,
    A_wo: jax.Array,
    B_x: jax.Array,
    B_W_gate: jax.Array,
    B_W_up: jax.Array,
    B_W_down: jax.Array,
    gate_w: jax.Array,
):
    B, S, D = A_x.shape
    assert B == 1
    Dh = A_wk.shape[1]
    H = A_wq.shape[1] // Dh
    F = B_W_gate.shape[1]

    kernel, scratch = _make_kernel(S, D, H, Dh, F)
    any_spec = pl.BlockSpec(memory_space=pl.ANY)
    out = pl.pallas_call(
        kernel,
        in_specs=[any_spec] * 9,
        out_specs=any_spec,
        out_shape=jax.ShapeDtypeStruct((S, D), A_x.dtype),
        scratch_shapes=scratch,
        compiler_params=pltpu.CompilerParams(
            vmem_limit_bytes=120 * 1024 * 1024,
        ),
    )(A_x.reshape(S, D), A_wq, A_wk.T, A_wv.T, A_wo, B_W_gate, B_W_up, B_W_down,
      gate_w.reshape(D // 128, 128))
    return out.reshape(B, S, D)
```

```python
import math

import jax
import jax.numpy as jnp
from jax import lax
import jax.experimental.pallas as pl
import jax.experimental.pallas.tpu as pltpu

_F32 = jnp.float32
_BF16 = jnp.bfloat16
_U32 = jnp.uint32

_TM = 128
_W = 256
_KC = 128
_G = 8
_FS = 256
_OR = 256
_OC = 128
_NV = 256
_SA = (0, 0, 1, 1, 2, 1, 2, 1, 1, 1, 2, 1, 1, 0, 0, 0)
_PF = (2, 3)
_DUE = 3
_C0 = 1
_LATE = 512
_LAST = 128
_PARK = 128
_HOLD = 4

_NT = (((1,), (1,)), ((), ()))


def _tree(op, parts):
    cur = list(parts)
    while len(cur) > 1:
        nxt = [op(cur[2 * j], cur[2 * j + 1]) for j in range(len(cur) // 2)]
        if len(cur) % 2:
            nxt.append(cur[-1])
        cur = nxt
    return cur[0]


def _b(u):
    return pltpu.bitcast(u, _BF16)


def _u(b):
    return pltpu.bitcast(b, _U32)


def _zero_of(v):
    return jnp.minimum(jnp.maximum(v, 0.0), 0.0)


def _make_kernel(S, D, H, Dh, F):
    W, KC, G, TM, NV = _W, _KC, _G, _TM, _NV
    NB = H * (S // W)
    NC = S // KC
    R = KC // 8
    LT = W // 128
    HD = H * Dh
    SM = S - NV
    NF = S // TM
    NG = NB // G
    GF = NG // NF
    FP = F // GF
    NJ = FP // _FS
    assert NV % 16 == 0 and H % G == 0 and NG % NF == 0 and F % (_FS * GF) == 0
    assert len(_SA) == NC and S == 2048 and W == 256 and _OR == W and HD % 1024 == 0

    a_steps = [n for n in range(1, G * NC) if _SA[n % NC]]
    NA = len(a_steps)
    pieces = []
    for e in range(G):
        for j in range(LT):
            kk = 0
            while kk < NV:
                n = len(pieces)
                size = _SA[a_steps[n] % NC] if n < NA else _PF[(n - NA) % len(_PF)]
                kb = min(8 * size, NV - kk)
                pieces.append((e, kk, kb, j))
                kk += kb
    assert all(p[0] == 0 or a_steps[t] >= (p[0] + 1) * NC for t, p in enumerate(pieces[:NA]))

    base, n_big = divmod(SM // 16, NC)
    big = set((NC * t) // n_big for t in range(n_big))
    qk_rows = [16 * (base + (c in big)) for c in range(NC)]
    assert all(sum(qk_rows[:c + 1]) <= KC * (c + 1) for c in range(NC))
    qk_start = [sum(qk_rows[:c]) for c in range(NC)]
    q_scale = (Dh ** -0.5) * math.log2(math.e)
    x_pieces = [(0, 256), (256, 256), (512, 512), (1024, 512), (1536, 512)]
    QC = HD // 4
    out_pieces = [(0, S - _LATE), (S - _LATE, _LATE - _LAST), (S - _LAST, _LAST)]
    GR = 16
    V0 = Dh + GR

    def kernel(x_hbm, wq_hbm, wkt_hbm, wvt_hbm, wo_hbm, wg_hbm, wu_hbm, wd_hbm, gw_hbm,
               out_hbm,
               x_u, wq_u, wkvt_u, wo_u, wg_u, wu_u, wd_u, gw_v,
               qt_u, k_u, vt_u, ot_u, o_u, out_v,
               kb_v, sv_v, vm_v, b_v, g_v, bs_v, park_v,
               xsems, qsems, wsems, osems, *bufs):
        sbufs = bufs[:G]
        mbufs = bufs[G:]
        x_h, wq_h, wkt_h, wvt_h, wo_h, wg_h, wu_h, wd_h = [
            r.bitcast(_U32) for r in
            (x_hbm, wq_hbm, wkt_hbm, wvt_hbm, wo_hbm, wg_hbm, wu_hbm, wd_hbm)]

        def x_copy(i):
            r0, n = x_pieces[i]
            rows = pl.ds(r0 // 2, n // 2)
            return pltpu.make_async_copy(x_h.at[rows], x_u.at[rows], xsems.at[i])

        def wq_copy(j):
            return pltpu.make_async_copy(
                wq_h.at[:, pl.ds(j * QC, QC)], wq_u.at[:, pl.ds(j * QC, QC)], qsems.at[j])

        w_pairs = [(wkt_h, wkvt_u.at[pl.ds(0, Dh // 2)]),
                   (wvt_h, wkvt_u.at[pl.ds(V0 // 2, Dh // 2)]),
                   (gw_hbm, gw_v)]
        for part in range(GF):
            fc = pl.ds(part * FP, FP)
            w_pairs += [(wg_h.at[:, fc], wg_u.at[part]), (wu_h.at[:, fc], wu_u.at[part]),
                        (wd_h.at[pl.ds(part * FP // 2, FP // 2)], wd_u.at[part])]
        w_pairs.append((wo_h, wo_u))

        def w_copy(j):
            return pltpu.make_async_copy(w_pairs[j][0], w_pairs[j][1], wsems.at[j])

        def out_copy(t):
            r0, n = out_pieces[t]
            return pltpu.make_async_copy(
                out_v.at[pl.ds(r0, n)], out_hbm.at[pl.ds(r0, n)], osems.at[t])

        def vpu_piece(qblk, slot, kk, kb, j, z):
            acc = z if kb == 8 else jnp.concatenate([z] * (kb // 8), axis=0)
            for d in range(Dh):
                t = kb_v[d, kk:kk + kb, :] * jnp.broadcast_to(qblk[d:d + 1, :], (kb, 128))
                acc = t + acc if d == 0 else acc + t
            sv_v[slot, kk:kk + kb, j * 128:(j + 1) * 128] = acc
            rows = [acc[r:r + 8, :] for r in range(0, kb, 8)]
            return _tree(jnp.maximum, rows), rows[0]

        def make_chain(grp):
            cs = dict(last=None, mv=None, q=None, done=0)

            def emit(upto):
                while cs["done"] < min(upto, len(pieces)):
                    e, kk, kb, j = pieces[cs["done"]]
                    slot = G if e == 0 else e
                    if kk == 0:
                        cs["q"] = _b(qt_u[grp * G + e])[:, j * 128:(j + 1) * 128].astype(_F32)
                    mxv, cs["last"] = vpu_piece(cs["q"], slot, kk, kb, j, _zero_of(cs["last"]))
                    cs["mv"] = mxv if kk == 0 else jnp.maximum(cs["mv"], mxv)
                    if kk + kb == NV:
                        vm_v[slot, :, j * 128:(j + 1) * 128] = cs["mv"]
                    cs["done"] += 1
            return cs, emit

        def attn_group(q_next, b_cur0, fillers=(), chain=None):
            do_qk = q_next is not None
            do_pv = b_cur0 is not None
            fillers = list(fillers)
            nfill = len(fillers)
            done = 0
            st = dict(mx=None, qt=None, m=None, acc=None, l=None)
            taps = []

            def load_scores(g, c):
                lo, hi = c * KC, (c + 1) * KC
                parts = []
                if lo < SM:
                    parts.append(sbufs[g][lo:min(hi, SM), :])
                if hi > SM:
                    parts.append(sv_v[g, max(lo, SM) - SM:hi - SM, :])
                sc = parts[0] if len(parts) == 1 else jnp.concatenate(parts, axis=0)
                if c == 0:
                    m = jnp.max(jnp.maximum(mbufs[g][...], vm_v[g]), axis=0, keepdims=True)
                    st["m"] = jnp.broadcast_to(m, (8, W))
                return sc.reshape(R, 8, W), st["m"]

            def qk(g, c):
                if c == 0:
                    st["qt"] = _b(q_next[g])
                    st["mx"] = None
                r0, n = qk_start[c], qk_rows[c]
                kc = _b(k_u[r0 // 2:(r0 + n) // 2, :])
                s = jnp.dot(kc, st["qt"], preferred_element_type=_F32)
                sbufs[g][r0:r0 + n, :] = s
                for r in range(0, n, 8):
                    sr = s[r:r + 8, :]
                    st["mx"] = sr if st["mx"] is None else jnp.maximum(st["mx"], sr)
                if c == NC - 1:
                    mbufs[g][...] = st["mx"]

            def pv(g, c, sc, m):
                lo, hi = c * KC, (c + 1) * KC
                if chain is not None:
                    ready = [v for (due, v) in taps if due <= g * NC + c]
                    taps[:] = [t for t in taps if t[0] > g * NC + c]
                    if c >= _C0:
                        link = st["l"]
                        if ready:
                            head = _tree(jnp.add, [link[:, :128]] + ready)
                            link = jnp.concatenate([head, link[:, 128:]], axis=1)
                        m = m + _zero_of(link)
                    elif ready:
                        head = m[:, :128] + _zero_of(_tree(jnp.add, ready))
                        m = jnp.concatenate([head, m[:, 128:]], axis=1)
                p = jnp.exp2(sc - m[None]).reshape(KC, W)
                t = _tree(jnp.add, [p[r:r + 8, :] for r in range(0, KC, 8)])
                st["l"] = t if c == 0 else st["l"] + t
                pb = p.astype(_BF16)
                d = jnp.dot(_b(vt_u[:, lo:hi]), pb, preferred_element_type=_F32)
                st["acc"] = d if c == 0 else st["acc"] + d
                if c == NC - 1:
                    lt = jnp.sum(st["l"], axis=0, keepdims=True)
                    ot_u[b_cur0 + g] = _u((st["acc"] * (1.0 / lt)).astype(_BF16))

            steps = [(g, c) for g in range(G) for c in range(NC)]
            pend = []
            for n, (g, c) in enumerate(steps):
                if do_pv:
                    pend.append((g, c) + load_scores(g, c))
                if do_qk:
                    qk(g, c)
                while done < nfill and done * len(steps) <= nfill * n:
                    fillers[done]()
                    done += 1
                if len(pend) > (1 if do_qk else 0):
                    pv(*pend.pop(0))
                if chain is not None and n in a_steps:
                    chain[0]["last"] = st["l"][:, :128]
                    chain[1](chain[0]["done"] + 1)
                    taps.append((n + _DUE, chain[0]["last"]))
            while pend:
                pv(*pend.pop(0))
            if chain is not None:
                chain[0]["last"] = st["l"][:, :128]
            while done < nfill:
                fillers[done]()
                done += 1

        def x_rows(r0, n):
            return _b(x_u[r0 // 2:(r0 + n) // 2, :])

        def kv_proj(r0, n):
            rows = slice(r0, r0 + n)
            kvt = lax.dot_general(_b(wkvt_u[...]), x_rows(r0, n), _NT,
                                  preferred_element_type=_F32)
            vt_u[:, rows] = _u(kvt[V0:, :].astype(_BF16))
            kg = jnp.concatenate([kvt[:Dh, :], jax.nn.sigmoid(kvt[Dh:Dh + 8, :])], axis=0).T
            k_u[r0 // 2:(r0 + n) // 2, :] = _u(kg[:, :Dh].astype(_BF16))
            g_v[rows, :] = kg[:, Dh:Dh + 1]

        def q_store(q, r0, n, c0, nc):
            qtb = q.T.astype(_BF16)
            for o in range(0, n, W):
                for h in range(c0 // Dh, (c0 + nc) // Dh):
                    hr = slice(h * Dh - c0, (h + 1) * Dh - c0)
                    qt_u[((r0 + o) // W) * H + h] = _u(qtb[hr, o:o + W])

        def q_mm(r0, n, c0, nc):
            return jnp.dot(x_rows(r0, n), _b(wq_u[:, c0:c0 + nc]),
                           preferred_element_type=_F32) * q_scale

        def q_proj(r0, n, c0, nc):
            q_store(q_mm(r0, n, c0, nc), r0, n, c0, nc)

        def q_proj_parked(r0, n, c0, nc):
            if nc > _PARK:
                q_proj(r0, n, c0, nc - _PARK)
            c1 = c0 + nc - _PARK
            park_v[0:n, :] = q_mm(r0, n, c1, _PARK)
            return lambda: q_store(park_v[0:n, :], r0, n, c1, _PARK)

        x_copy(0).start()
        for j in range(3):
            w_copy(j).start()
        wq_copy(0).start()
        wq_copy(1).start()
        bs_v[...] = jnp.zeros_like(bs_v)
        x_copy(0).wait()
        for j in range(3):
            w_copy(j).wait()
        x_copy(1).start()
        gw = gw_v[...].astype(_F32)
        first_row = lax.broadcasted_iota(jnp.int32, (GR, 128), 0) == 0
        for c in range(D // 128):
            tile = jnp.where(first_row, jnp.broadcast_to(gw[c:c + 1, :], (GR, 128)), 0.0)
            wkvt_u[Dh // 2:V0 // 2, c * 128:(c + 1) * 128] = _u(tile.astype(_BF16))
        kv_proj(0, 256)
        wq_copy(0).wait()
        wq_copy(2).start()
        finish = q_proj_parked(0, 256, 0, QC)
        wq_copy(1).wait()
        wq_copy(3).start()
        finish()
        finish = q_proj_parked(0, 256, QC, QC)
        x_copy(1).wait()
        x_copy(2).start()
        finish()
        kv_proj(256, 256)
        finish = q_proj_parked(256, 256, 0, 2 * QC)
        wq_copy(2).wait()
        wq_copy(3).wait()
        x_copy(3).start()
        x_copy(4).start()
        finish()
        finish = q_proj_parked(0, 512, 2 * QC, 2 * QC)
        x_copy(2).wait()
        for j in range(3, len(w_pairs)):
            w_copy(j).start()
        finish()
        kv_proj(512, 512)
        finish = q_proj_parked(512, 512, 0, HD)
        x_copy(3).wait()
        x_copy(4).wait()
        finish()
        kv_proj(1024, 512)
        kv_proj(1536, 512)
        for r0 in (1024, 1536):
            q_proj(r0, 512, 0, HD)
        kf = _b(k_u[SM // 2:, :]).astype(_F32)
        for d in range(Dh):
            kb_v[d] = jnp.broadcast_to(kf[:, d:d + 1], (NV, 128))

        attn_group(qt_u, None)
        kc = _b(k_u[SM // 2:, :])
        for g in range(G):
            s = jnp.dot(kc, _b(qt_u[g]), preferred_element_type=_F32)
            sv_v[g] = s
            s3 = s.reshape(NV // 8, 8, W)
            vm_v[g] = _tree(jnp.maximum, [s3[r] for r in range(NV // 8)])

        def ffn_part(q, chain):
            i = q // GF
            part = q % GF
            rows = pl.ds(pl.multiple_of(i * TM, TM), TM)
            items = []
            for j in range(NJ + 1):
                if j < NJ:
                    items.append(("gu", j, 2))
                if j >= 1:
                    items.append(("d", j - 1, 1))
            total = sum(it[2] for it in items)
            accum = 0
            hid = {}
            xt = _b(x_u[pl.ds(pl.multiple_of(i * (TM // 2), TM // 2), TM // 2), :])
            nf = len(pieces) - NA
            moved = False
            for kind, j, cost in items:
                cols = slice(j * _FS, (j + 1) * _FS)
                if kind == "gu":
                    gate = jnp.dot(xt, _b(wg_u[part, :, cols]), preferred_element_type=_F32)
                    up = jnp.dot(xt, _b(wu_u[part, :, cols]), preferred_element_type=_F32)
                    hid[j] = (jnp.maximum(gate, 0.0) * up).astype(_BF16)
                else:
                    wd = _b(wd_u[part, j * _FS // 2:(j + 1) * _FS // 2, :])
                    dv = jnp.dot(hid.pop(j), wd, preferred_element_type=_F32)
                    if j == 0:
                        bs_v[...] = jnp.where(part == 0, 0.0, bs_v[...]) + dv
                    elif j == NJ - 1:
                        tot = bs_v[...] + dv
                        bs_v[...] = tot
                        b_v[rows, :] = tot
                    else:
                        bs_v[...] += dv
                accum += cost
                chain[1](NA + (nf * accum + total - 1) // total)
                if not moved and pieces[min(chain[0]["done"], len(pieces) - 1)][0] > 0:
                    sv_v[0] = sv_v[G]
                    vm_v[0] = vm_v[G]
                    moved = True

        for j in range(3, 6):
            w_copy(j).wait()

        def main_body(q, carry):
            for part in range(1, GF):
                @pl.when(q == part)
                def _():
                    for j in range(3 + 3 * part, 6 + 3 * part):
                        w_copy(j).wait()

            chain = make_chain(q + 1)
            attn_group(qt_u.at[pl.ds((q + 1) * G, G)], q * G, chain=chain)
            ffn_part(q, chain)
            return carry

        lax.fori_loop(0, NG - 1, main_body, 0)

        w_copy(len(w_pairs) - 1).wait()

        def transpose_o(r0, n):
            lanes = slice(r0 % W, r0 % W + n)
            ot = jnp.concatenate(
                [_b(ot_u[(r0 // W) * H + h, :, lanes]) for h in range(H)], axis=0)
            o_u[r0 // 2:(r0 + n) // 2, :] = _u(ot.T)

        def oproj_piece(r0, n, c0, nc, prep):
            def f():
                rows = slice(r0, r0 + n)
                cols = slice(c0, c0 + nc)
                if prep:
                    transpose_o(r0, n)
                a = jnp.dot(_b(o_u[r0 // 2:(r0 + n) // 2, :]), _b(wo_u[:, cols]),
                            preferred_element_type=_F32)
                g = g_v[rows, :]
                out_v[rows, cols] = (g * a + (1.0 - g) * b_v[rows, cols]).astype(_BF16)
            return f

        def oproj_rows(lo, hi, prep):
            fs = []
            r0 = lo
            while r0 < hi:
                n = min(_OR, hi - r0)
                nc = _OC * _OR // n
                fs += [oproj_piece(r0, n, c0, nc, prep and c0 == 0) for c0 in range(0, D, nc)]
                r0 += n
            return fs

        def last_ffn_items():
            rows = slice(S - TM, S)
            hid = {}
            fs = []

            def gate(j):
                def f():
                    cols = slice(j * _FS, (j + 1) * _FS)
                    hid[j] = jnp.dot(x_rows(S - TM, TM), _b(wg_u[GF - 1, :, cols]),
                                     preferred_element_type=_F32)
                return f

            def up(j):
                def f():
                    cols = slice(j * _FS, (j + 1) * _FS)
                    u = jnp.dot(x_rows(S - TM, TM), _b(wu_u[GF - 1, :, cols]),
                                preferred_element_type=_F32)
                    hid[j] = (jnp.maximum(hid[j], 0.0) * u).astype(_BF16)
                return f

            def down(j):
                def f():
                    wd = _b(wd_u[GF - 1, j * _FS // 2:(j + 1) * _FS // 2, :])
                    dv = jnp.dot(hid.pop(j), wd, preferred_element_type=_F32)
                    b_v[rows, :] += dv
                return f

            for j in range(NJ + 1):
                if j < NJ:
                    fs += [gate(j), up(j)]
                if j >= 1:
                    fs.append(down(j - 1))
            return fs

        fill = last_ffn_items() + oproj_rows(0, S - _LATE, True)
        attn_group(None, NB - G, fill[:len(fill) - _HOLD])
        for r0 in range(S - _LATE, S, _OR):
            transpose_o(r0, _OR)
        for f in fill[len(fill) - _HOLD:]:
            f()
        out_copy(0).start()
        for t in range(1, len(out_pieces)):
            r0, n = out_pieces[t]
            for f in oproj_rows(r0, r0 + n, False):
                f()
            out_copy(t).start()
        for t in range(len(out_pieces)):
            out_copy(t).wait()

    scratch = [
        pltpu.VMEM((S // 2, D), _U32),
        pltpu.VMEM((D // 2, HD), _U32),
        pltpu.VMEM(((V0 + Dh) // 2, D), _U32),
        pltpu.VMEM((HD // 2, D), _U32),
        pltpu.VMEM((GF, D // 2, FP), _U32),
        pltpu.VMEM((GF, D // 2, FP), _U32),
        pltpu.VMEM((GF, FP // 2, D), _U32),
        pltpu.VMEM((D // 128, 128), _BF16),
        pltpu.VMEM((NB, Dh // 2, W), _U32),
        pltpu.VMEM((S // 2, Dh), _U32),
        pltpu.VMEM((Dh // 2, S), _U32),
        pltpu.VMEM((NB, Dh // 2, W), _U32),
        pltpu.VMEM((S // 2, HD), _U32),
        pltpu.VMEM((S, D), _BF16),
        pltpu.VMEM((Dh, NV, 128), _F32),
        pltpu.VMEM((G + 1, NV, W), _F32),
        pltpu.VMEM((G + 1, 8, W), _F32),
        pltpu.VMEM((S, D), _F32),
        pltpu.VMEM((S, 1), _F32),
        pltpu.VMEM((TM, D), _F32),
        pltpu.VMEM((512, _PARK), _F32),
        pltpu.SemaphoreType.DMA((len(x_pieces),)),
        pltpu.SemaphoreType.DMA((4,)),
        pltpu.SemaphoreType.DMA((4 + 3 * GF,)),
        pltpu.SemaphoreType.DMA((len(out_pieces),)),
    ] + [pltpu.VMEM((SM, W), _F32)] * G + [pltpu.VMEM((8, W), _F32)] * G
    return kernel, scratch


@jax.jit
def pallas_gated_mix__grouped_kv_mqa__glu_gated_reglu__prompt_kernel(
    A_x: jax.Array,
    A_wq: jax.Array,
    A_wk: jax.Array,
    A_wv: jax.Array,
    A_wo: jax.Array,
    B_x: jax.Array,
    B_W_gate: jax.Array,
    B_W_up: jax.Array,
    B_W_down: jax.Array,
    gate_w: jax.Array,
):
    B, S, D = A_x.shape
    assert B == 1
    Dh = A_wk.shape[1]
    H = A_wq.shape[1] // Dh
    F = B_W_gate.shape[1]

    kernel, scratch = _make_kernel(S, D, H, Dh, F)
    any_spec = pl.BlockSpec(memory_space=pl.ANY)
    out = pl.pallas_call(
        kernel,
        in_specs=[any_spec] * 9,
        out_specs=any_spec,
        out_shape=jax.ShapeDtypeStruct((S, D), A_x.dtype),
        scratch_shapes=scratch,
        compiler_params=pltpu.CompilerParams(
            vmem_limit_bytes=120 * 1024 * 1024,
        ),
    )(A_x.reshape(S, D), A_wq, A_wk.T, A_wv.T, A_wo, B_W_gate, B_W_up, B_W_down,
      gate_w.reshape(D // 128, 128))
    return out.reshape(B, S, D)
```

```python
import math

import jax
import jax.numpy as jnp
from jax import lax
import jax.experimental.pallas as pl
import jax.experimental.pallas.tpu as pltpu

_F32 = jnp.float32
_BF16 = jnp.bfloat16
_U32 = jnp.uint32

_TM = 128
_W = 256
_KC = 128
_G = 8
_FS = 256
_OR = 256
_OC = 128
_NV = 256
_SA = (0, 0, 1, 1, 2, 1, 2, 1, 1, 1, 2, 1, 1, 0, 0, 0)
_PF = (2, 3)
_DUE = 3
_C0 = 1
_LATE = 512
_LAST = 128
_PARK = 128
_HOLD = 4

_NT = (((1,), (1,)), ((), ()))


def _tree(op, parts):
    cur = list(parts)
    while len(cur) > 1:
        nxt = [op(cur[2 * j], cur[2 * j + 1]) for j in range(len(cur) // 2)]
        if len(cur) % 2:
            nxt.append(cur[-1])
        cur = nxt
    return cur[0]


def _b(u):
    return pltpu.bitcast(u, _BF16)


def _u(b):
    return pltpu.bitcast(b, _U32)


def _zero_of(v):
    return jnp.minimum(jnp.maximum(v, 0.0), 0.0)


def _make_kernel(S, D, H, Dh, F):
    W, KC, G, TM, NV = _W, _KC, _G, _TM, _NV
    NB = H * (S // W)
    NC = S // KC
    R = KC // 8
    LT = W // 128
    HD = H * Dh
    SM = S - NV
    NF = S // TM
    NG = NB // G
    GF = NG // NF
    FP = F // GF
    NJ = FP // _FS
    assert NV % 16 == 0 and H % G == 0 and NG % NF == 0 and F % (_FS * GF) == 0
    assert len(_SA) == NC and S == 2048 and W == 256 and _OR == W and HD % 1024 == 0

    a_steps = [n for n in range(1, G * NC) if _SA[n % NC]]
    NA = len(a_steps)
    pieces = []
    for e in range(G):
        for j in range(LT):
            kk = 0
            while kk < NV:
                n = len(pieces)
                size = _SA[a_steps[n] % NC] if n < NA else _PF[(n - NA) % len(_PF)]
                kb = min(8 * size, NV - kk)
                pieces.append((e, kk, kb, j))
                kk += kb
    assert all(p[0] == 0 or a_steps[t] >= (p[0] + 1) * NC for t, p in enumerate(pieces[:NA]))

    base, n_big = divmod(SM // 16, NC)
    big = set((NC * t) // n_big for t in range(n_big))
    qk_rows = [16 * (base + (c in big)) for c in range(NC)]
    assert all(sum(qk_rows[:c + 1]) <= KC * (c + 1) for c in range(NC))
    qk_start = [sum(qk_rows[:c]) for c in range(NC)]
    q_scale = (Dh ** -0.5) * math.log2(math.e)
    x_pieces = [(0, 256), (256, 256), (512, 512), (1024, 512), (1536, 512)]
    QC = HD // 4
    out_pieces = [(r0, _OR) for r0 in range(0, S - _OR, _OR)]
    out_pieces += [(r0, _LAST) for r0 in range(S - _OR, S, _LAST)]
    assert len(out_pieces) <= len(x_pieces) + 4
    GR = 16
    V0 = Dh + GR

    def kernel(x_hbm, wq_hbm, wkt_hbm, wvt_hbm, wo_hbm, wg_hbm, wu_hbm, wd_hbm, gw_hbm,
               out_hbm,
               x_u, wq_u, wkvt_u, wo_u, wg_u, wu_u, wd_u, gw_v,
               qt_u, k_u, vt_u, ot_u, o_u, out_v,
               kb_v, sv_v, vm_v, b_v, g_v, bs_v, park_v,
               xsems, qsems, wsems, *bufs):
        sbufs = bufs[:G]
        mbufs = bufs[G:]
        x_h, wq_h, wkt_h, wvt_h, wo_h, wg_h, wu_h, wd_h = [
            r.bitcast(_U32) for r in
            (x_hbm, wq_hbm, wkt_hbm, wvt_hbm, wo_hbm, wg_hbm, wu_hbm, wd_hbm)]

        def x_copy(i):
            r0, n = x_pieces[i]
            rows = pl.ds(r0 // 2, n // 2)
            return pltpu.make_async_copy(x_h.at[rows], x_u.at[rows], xsems.at[i])

        def wq_copy(j):
            return pltpu.make_async_copy(
                wq_h.at[:, pl.ds(j * QC, QC)], wq_u.at[:, pl.ds(j * QC, QC)], qsems.at[j])

        w_pairs = [(wkt_h, wkvt_u.at[pl.ds(0, Dh // 2)]),
                   (wvt_h, wkvt_u.at[pl.ds(V0 // 2, Dh // 2)]),
                   (gw_hbm, gw_v)]
        for part in range(GF):
            fc = pl.ds(part * FP, FP)
            w_pairs += [(wg_h.at[:, fc], wg_u.at[part]), (wu_h.at[:, fc], wu_u.at[part]),
                        (wd_h.at[pl.ds(part * FP // 2, FP // 2)], wd_u.at[part])]
        w_pairs.append((wo_h, wo_u))

        def w_copy(j):
            return pltpu.make_async_copy(w_pairs[j][0], w_pairs[j][1], wsems.at[j])

        def out_copy(t):
            r0, n = out_pieces[t]
            sem = xsems.at[t] if t < len(x_pieces) else qsems.at[t - len(x_pieces)]
            return pltpu.make_async_copy(out_v.at[pl.ds(r0, n)], out_hbm.at[pl.ds(r0, n)], sem)

        def vpu_piece(qblk, slot, kk, kb, j, z):
            acc = z if kb == 8 else jnp.concatenate([z] * (kb // 8), axis=0)
            for d in range(Dh):
                t = kb_v[d, kk:kk + kb, :] * jnp.broadcast_to(qblk[d:d + 1, :], (kb, 128))
                acc = t + acc if d == 0 else acc + t
            sv_v[slot, kk:kk + kb, j * 128:(j + 1) * 128] = acc
            rows = [acc[r:r + 8, :] for r in range(0, kb, 8)]
            return _tree(jnp.maximum, rows), rows[0]

        def make_chain(grp):
            cs = dict(last=None, mv=None, q=None, done=0)

            def emit(upto):
                while cs["done"] < min(upto, len(pieces)):
                    e, kk, kb, j = pieces[cs["done"]]
                    slot = G if e == 0 else e
                    if kk == 0:
                        cs["q"] = _b(qt_u[grp * G + e])[:, j * 128:(j + 1) * 128].astype(_F32)
                    mxv, cs["last"] = vpu_piece(cs["q"], slot, kk, kb, j, _zero_of(cs["last"]))
                    cs["mv"] = mxv if kk == 0 else jnp.maximum(cs["mv"], mxv)
                    if kk + kb == NV:
                        vm_v[slot, :, j * 128:(j + 1) * 128] = cs["mv"]
                    cs["done"] += 1
            return cs, emit

        def attn_group(q_next, b_cur0, fillers=(), chain=None):
            do_qk = q_next is not None
            do_pv = b_cur0 is not None
            fillers = list(fillers)
            nfill = len(fillers)
            done = 0
            st = dict(mx=None, qt=None, m=None, acc=None, l=None)
            taps = []

            def load_scores(g, c):
                lo, hi = c * KC, (c + 1) * KC
                parts = []
                if lo < SM:
                    parts.append(sbufs[g][lo:min(hi, SM), :])
                if hi > SM:
                    parts.append(sv_v[g, max(lo, SM) - SM:hi - SM, :])
                sc = parts[0] if len(parts) == 1 else jnp.concatenate(parts, axis=0)
                if c == 0:
                    m = jnp.max(jnp.maximum(mbufs[g][...], vm_v[g]), axis=0, keepdims=True)
                    st["m"] = jnp.broadcast_to(m, (8, W))
                return sc.reshape(R, 8, W), st["m"]

            def qk(g, c):
                if c == 0:
                    st["qt"] = _b(q_next[g])
                    st["mx"] = None
                r0, n = qk_start[c], qk_rows[c]
                kc = _b(k_u[r0 // 2:(r0 + n) // 2, :])
                s = jnp.dot(kc, st["qt"], preferred_element_type=_F32)
                sbufs[g][r0:r0 + n, :] = s
                for r in range(0, n, 8):
                    sr = s[r:r + 8, :]
                    st["mx"] = sr if st["mx"] is None else jnp.maximum(st["mx"], sr)
                if c == NC - 1:
                    mbufs[g][...] = st["mx"]

            def pv(g, c, sc, m):
                lo, hi = c * KC, (c + 1) * KC
                if chain is not None:
                    ready = [v for (due, v) in taps if due <= g * NC + c]
                    taps[:] = [t for t in taps if t[0] > g * NC + c]
                    if c >= _C0:
                        link = st["l"]
                        if ready:
                            head = _tree(jnp.add, [link[:, :128]] + ready)
                            link = jnp.concatenate([head, link[:, 128:]], axis=1)
                        m = m + _zero_of(link)
                    elif ready:
                        head = m[:, :128] + _zero_of(_tree(jnp.add, ready))
                        m = jnp.concatenate([head, m[:, 128:]], axis=1)
                p = jnp.exp2(sc - m[None]).reshape(KC, W)
                t = _tree(jnp.add, [p[r:r + 8, :] for r in range(0, KC, 8)])
                st["l"] = t if c == 0 else st["l"] + t
                pb = p.astype(_BF16)
                d = jnp.dot(_b(vt_u[:, lo:hi]), pb, preferred_element_type=_F32)
                st["acc"] = d if c == 0 else st["acc"] + d
                if c == NC - 1:
                    lt = jnp.sum(st["l"], axis=0, keepdims=True)
                    ot_u[b_cur0 + g] = _u((st["acc"] * (1.0 / lt)).astype(_BF16))

            steps = [(g, c) for g in range(G) for c in range(NC)]
            pend = []
            for n, (g, c) in enumerate(steps):
                if do_pv:
                    pend.append((g, c) + load_scores(g, c))
                if do_qk:
                    qk(g, c)
                while done < nfill and done * len(steps) <= nfill * n:
                    fillers[done]()
                    done += 1
                if len(pend) > (1 if do_qk else 0):
                    pv(*pend.pop(0))
                if chain is not None and n in a_steps:
                    chain[0]["last"] = st["l"][:, :128]
                    chain[1](chain[0]["done"] + 1)
                    taps.append((n + _DUE, chain[0]["last"]))
            while pend:
                pv(*pend.pop(0))
            if chain is not None:
                chain[0]["last"] = st["l"][:, :128]
            while done < nfill:
                fillers[done]()
                done += 1

        def x_rows(r0, n):
            return _b(x_u[r0 // 2:(r0 + n) // 2, :])

        def kv_proj(r0, n):
            rows = slice(r0, r0 + n)
            kvt = lax.dot_general(_b(wkvt_u[...]), x_rows(r0, n), _NT,
                                  preferred_element_type=_F32)
            vt_u[:, rows] = _u(kvt[V0:, :].astype(_BF16))
            kg = jnp.concatenate([kvt[:Dh, :], jax.nn.sigmoid(kvt[Dh:Dh + 8, :])], axis=0).T
            k_u[r0 // 2:(r0 + n) // 2, :] = _u(kg[:, :Dh].astype(_BF16))
            g_v[rows, :] = kg[:, Dh:Dh + 1]

        def q_store(q, r0, n, c0, nc):
            qtb = q.T.astype(_BF16)
            for o in range(0, n, W):
                for h in range(c0 // Dh, (c0 + nc) // Dh):
                    hr = slice(h * Dh - c0, (h + 1) * Dh - c0)
                    qt_u[((r0 + o) // W) * H + h] = _u(qtb[hr, o:o + W])

        def q_mm(r0, n, c0, nc):
            return jnp.dot(x_rows(r0, n), _b(wq_u[:, c0:c0 + nc]),
                           preferred_element_type=_F32) * q_scale

        def q_proj(r0, n, c0, nc):
            q_store(q_mm(r0, n, c0, nc), r0, n, c0, nc)

        def q_proj_parked(r0, n, c0, nc):
            if nc > _PARK:
                q_proj(r0, n, c0, nc - _PARK)
            c1 = c0 + nc - _PARK
            park_v[0:n, :] = q_mm(r0, n, c1, _PARK)
            return lambda: q_store(park_v[0:n, :], r0, n, c1, _PARK)

        x_copy(0).start()
        for j in range(3):
            w_copy(j).start()
        wq_copy(0).start()
        wq_copy(1).start()
        bs_v[...] = jnp.zeros_like(bs_v)
        x_copy(0).wait()
        for j in range(3):
            w_copy(j).wait()
        x_copy(1).start()
        gw = gw_v[...].astype(_F32)
        first_row = lax.broadcasted_iota(jnp.int32, (GR, 128), 0) == 0
        for c in range(D // 128):
            tile = jnp.where(first_row, jnp.broadcast_to(gw[c:c + 1, :], (GR, 128)), 0.0)
            wkvt_u[Dh // 2:V0 // 2, c * 128:(c + 1) * 128] = _u(tile.astype(_BF16))
        kv_proj(0, 256)
        wq_copy(0).wait()
        wq_copy(2).start()
        finish = q_proj_parked(0, 256, 0, QC)
        wq_copy(1).wait()
        wq_copy(3).start()
        finish()
        finish = q_proj_parked(0, 256, QC, QC)
        x_copy(1).wait()
        x_copy(2).start()
        finish()
        kv_proj(256, 256)
        finish = q_proj_parked(256, 256, 0, 2 * QC)
        wq_copy(2).wait()
        wq_copy(3).wait()
        x_copy(3).start()
        x_copy(4).start()
        finish()
        finish = q_proj_parked(0, 512, 2 * QC, 2 * QC)
        x_copy(2).wait()
        for j in range(3, len(w_pairs)):
            w_copy(j).start()
        finish()
        kv_proj(512, 512)
        finish = q_proj_parked(512, 512, 0, HD)
        x_copy(3).wait()
        x_copy(4).wait()
        finish()
        kv_proj(1024, 512)
        kv_proj(1536, 512)
        for r0 in (1024, 1536):
            q_proj(r0, 512, 0, HD)
        kf = _b(k_u[SM // 2:, :]).astype(_F32)
        for d in range(Dh):
            kb_v[d] = jnp.broadcast_to(kf[:, d:d + 1], (NV, 128))

        attn_group(qt_u, None)
        kc = _b(k_u[SM // 2:, :])
        for g in range(G):
            s = jnp.dot(kc, _b(qt_u[g]), preferred_element_type=_F32)
            sv_v[g] = s
            s3 = s.reshape(NV // 8, 8, W)
            vm_v[g] = _tree(jnp.maximum, [s3[r] for r in range(NV // 8)])

        def ffn_part(q, chain):
            i = q // GF
            part = q % GF
            rows = pl.ds(pl.multiple_of(i * TM, TM), TM)
            items = []
            for j in range(NJ + 1):
                if j < NJ:
                    items.append(("gu", j, 2))
                if j >= 1:
                    items.append(("d", j - 1, 1))
            total = sum(it[2] for it in items)
            accum = 0
            hid = {}
            xt = _b(x_u[pl.ds(pl.multiple_of(i * (TM // 2), TM // 2), TM // 2), :])
            nf = len(pieces) - NA
            moved = False
            for kind, j, cost in items:
                cols = slice(j * _FS, (j + 1) * _FS)
                if kind == "gu":
                    gate = jnp.dot(xt, _b(wg_u[part, :, cols]), preferred_element_type=_F32)
                    up = jnp.dot(xt, _b(wu_u[part, :, cols]), preferred_element_type=_F32)
                    hid[j] = (jnp.maximum(gate, 0.0) * up).astype(_BF16)
                else:
                    wd = _b(wd_u[part, j * _FS // 2:(j + 1) * _FS // 2, :])
                    dv = jnp.dot(hid.pop(j), wd, preferred_element_type=_F32)
                    if j == 0:
                        bs_v[...] = jnp.where(part == 0, 0.0, bs_v[...]) + dv
                    elif j == NJ - 1:
                        tot = bs_v[...] + dv
                        bs_v[...] = tot
                        b_v[rows, :] = tot
                    else:
                        bs_v[...] += dv
                accum += cost
                chain[1](NA + (nf * accum + total - 1) // total)
                if not moved and pieces[min(chain[0]["done"], len(pieces) - 1)][0] > 0:
                    sv_v[0] = sv_v[G]
                    vm_v[0] = vm_v[G]
                    moved = True

        for j in range(3, 6):
            w_copy(j).wait()

        def main_body(q, carry):
            for part in range(1, GF):
                @pl.when(q == part)
                def _():
                    for j in range(3 + 3 * part, 6 + 3 * part):
                        w_copy(j).wait()

            chain = make_chain(q + 1)
            attn_group(qt_u.at[pl.ds((q + 1) * G, G)], q * G, chain=chain)
            ffn_part(q, chain)
            return carry

        lax.fori_loop(0, NG - 1, main_body, 0)

        w_copy(len(w_pairs) - 1).wait()

        def transpose_o(r0, n):
            lanes = slice(r0 % W, r0 % W + n)
            ot = jnp.concatenate(
                [_b(ot_u[(r0 // W) * H + h, :, lanes]) for h in range(H)], axis=0)
            o_u[r0 // 2:(r0 + n) // 2, :] = _u(ot.T)

        def oproj_piece(t, c0, nc, prep):
            r0, n = out_pieces[t]

            def f():
                rows = slice(r0, r0 + n)
                cols = slice(c0, c0 + nc)
                if prep:
                    transpose_o(r0, n)
                a = jnp.dot(_b(o_u[r0 // 2:(r0 + n) // 2, :]), _b(wo_u[:, cols]),
                            preferred_element_type=_F32)
                g = g_v[rows, :]
                out_v[rows, cols] = (g * a + (1.0 - g) * b_v[rows, cols]).astype(_BF16)
                if c0 + nc == D:
                    out_copy(t).start()
            return f

        def oproj_rows(lo, hi, prep):
            fs = []
            for t, (r0, n) in enumerate(out_pieces):
                if lo <= r0 < hi:
                    nc = min(_OC * _OR // n, D)
                    fs += [oproj_piece(t, c0, nc, prep and c0 == 0) for c0 in range(0, D, nc)]
            return fs

        def last_ffn_items():
            rows = slice(S - TM, S)
            hid = {}
            fs = []

            def gate(j):
                def f():
                    cols = slice(j * _FS, (j + 1) * _FS)
                    hid[j] = jnp.dot(x_rows(S - TM, TM), _b(wg_u[GF - 1, :, cols]),
                                     preferred_element_type=_F32)
                return f

            def up(j):
                def f():
                    cols = slice(j * _FS, (j + 1) * _FS)
                    u = jnp.dot(x_rows(S - TM, TM), _b(wu_u[GF - 1, :, cols]),
                                preferred_element_type=_F32)
                    hid[j] = (jnp.maximum(hid[j], 0.0) * u).astype(_BF16)
                return f

            def down(j):
                def f():
                    wd = _b(wd_u[GF - 1, j * _FS // 2:(j + 1) * _FS // 2, :])
                    dv = jnp.dot(hid.pop(j), wd, preferred_element_type=_F32)
                    b_v[rows, :] += dv
                return f

            for j in range(NJ + 1):
                if j < NJ:
                    fs += [gate(j), up(j)]
                if j >= 1:
                    fs.append(down(j - 1))
            return fs

        fill = last_ffn_items() + oproj_rows(0, S - _LATE, True)
        attn_group(None, NB - G, fill[:len(fill) - _HOLD])
        for r0 in range(S - _LATE, S, _OR):
            transpose_o(r0, _OR)
        for f in fill[len(fill) - _HOLD:]:
            f()
        for f in oproj_rows(S - _LATE, S, False):
            f()
        for t in range(len(out_pieces)):
            out_copy(t).wait()

    scratch = [
        pltpu.VMEM((S // 2, D), _U32),
        pltpu.VMEM((D // 2, HD), _U32),
        pltpu.VMEM(((V0 + Dh) // 2, D), _U32),
        pltpu.VMEM((HD // 2, D), _U32),
        pltpu.VMEM((GF, D // 2, FP), _U32),
        pltpu.VMEM((GF, D // 2, FP), _U32),
        pltpu.VMEM((GF, FP // 2, D), _U32),
        pltpu.VMEM((D // 128, 128), _BF16),
        pltpu.VMEM((NB, Dh // 2, W), _U32),
        pltpu.VMEM((S // 2, Dh), _U32),
        pltpu.VMEM((Dh // 2, S), _U32),
        pltpu.VMEM((NB, Dh // 2, W), _U32),
        pltpu.VMEM((S // 2, HD), _U32),
        pltpu.VMEM((S, D), _BF16),
        pltpu.VMEM((Dh, NV, 128), _F32),
        pltpu.VMEM((G + 1, NV, W), _F32),
        pltpu.VMEM((G + 1, 8, W), _F32),
        pltpu.VMEM((S, D), _F32),
        pltpu.VMEM((S, 1), _F32),
        pltpu.VMEM((TM, D), _F32),
        pltpu.VMEM((512, _PARK), _F32),
        pltpu.SemaphoreType.DMA((len(x_pieces),)),
        pltpu.SemaphoreType.DMA((4,)),
        pltpu.SemaphoreType.DMA((4 + 3 * GF,)),
    ] + [pltpu.VMEM((SM, W), _F32)] * G + [pltpu.VMEM((8, W), _F32)] * G
    return kernel, scratch


@jax.jit
def pallas_gated_mix__grouped_kv_mqa__glu_gated_reglu__prompt_kernel(
    A_x: jax.Array,
    A_wq: jax.Array,
    A_wk: jax.Array,
    A_wv: jax.Array,
    A_wo: jax.Array,
    B_x: jax.Array,
    B_W_gate: jax.Array,
    B_W_up: jax.Array,
    B_W_down: jax.Array,
    gate_w: jax.Array,
):
    B, S, D = A_x.shape
    assert B == 1
    Dh = A_wk.shape[1]
    H = A_wq.shape[1] // Dh
    F = B_W_gate.shape[1]

    kernel, scratch = _make_kernel(S, D, H, Dh, F)
    any_spec = pl.BlockSpec(memory_space=pl.ANY)
    out = pl.pallas_call(
        kernel,
        in_specs=[any_spec] * 9,
        out_specs=any_spec,
        out_shape=jax.ShapeDtypeStruct((S, D), A_x.dtype),
        scratch_shapes=scratch,
        compiler_params=pltpu.CompilerParams(
            vmem_limit_bytes=120 * 1024 * 1024,
        ),
    )(A_x.reshape(S, D), A_wq, A_wk.T, A_wv.T, A_wo, B_W_gate, B_W_up, B_W_down,
      gate_w.reshape(D // 128, 128))
    return out.reshape(B, S, D)
```
